```python
import jax
import jax.numpy as jnp

def _softmax(x, axis=-1):
    return jax.nn.softmax(x, axis=axis)

def _gelu(x):
    return jax.nn.gelu(x, approximate=True)

def _silu(x):
    return jax.nn.silu(x)

def _sigmoid(x):
    return jax.nn.sigmoid(x)

def _layernorm(x, axis=-1, eps=1e-05):
    m = jnp.mean(x, axis=axis, keepdims=True)
    v = jnp.var(x, axis=axis, keepdims=True)
    return (x - m) / jnp.sqrt(v + eps)

def _scatter_add(tgt, idx, src, axis=0):
    return tgt.at[idx].add(src)

def _segment_sum(src, seg, n):
    return jax.ops.segment_sum(src, seg, n)

class _Rng:

    def __init__(self, key):
        self._k = key

    def _next(self):
        self._k, sub = jax.random.split(self._k)
        return sub

    def normal(self, shape):
        return jax.random.normal(self._next(), shape, dtype=jnp.bfloat16)

    def randint(self, lo, hi, shape):
        return jax.random.randint(self._next(), shape, lo, hi, dtype=jnp.int32)

    def uniform(self, shape, lo=0.0, hi=1.0):
        return jax.random.uniform(self._next(), shape, jnp.bfloat16, lo, hi)

    def permutation(self, n):
        return jax.random.permutation(self._next(), n)
kernel_name = 'sequential_preLN__memory_aug_infini_attn__moe_arch_mod__prompt'

def setup_inputs():
    _rng = _Rng(jax.random.key(int.from_bytes(__import__("os").urandom(4), "little")))
    _w = lambda a: (lambda t: t.astype(jnp.bfloat16) if jnp.issubdtype(t.dtype, jnp.floating) else t)(jnp.asarray(a))

    def _A_setup():
        B, S, D, H = (1, 2048, 576, 32)
        N = 4
        L = max(1, S // N)
        sc = D ** (-0.5)
        return {'x': _w((lambda *s: _rng.normal(s) * 0.05)(B, N * L, D)), 'wq': _w((lambda *s: _rng.normal(s) * 0.05)(D, D) * sc), 'wk': _w((lambda *s: _rng.normal(s) * 0.05)(D, D) * sc), 'wv': _w((lambda *s: _rng.normal(s) * 0.05)(D, D) * sc), 'wo': _w((lambda *s: _rng.normal(s) * 0.05)(D, D) * sc), 'beta': _w((lambda *s: _rng.normal(s) * 0.05)(H))}
    _A_in = _A_setup()

    def _B_setup():
        B, S, D, F, C = (1, 2048, 576, 4608, 1)
        return {'x': _w((lambda *s: _rng.normal(s) * 0.05)(B, S, D)), 'w_r': _w((lambda *s: _rng.normal(s) * 0.05)(D)), 'w_gate': _w((lambda *s: _rng.normal(s) * 0.05)(D, F)), 'w_up': _w((lambda *s: _rng.normal(s) * 0.05)(D, F)), 'w_down': _w((lambda *s: _rng.normal(s) * 0.05)(F, D))}
    _B_in = _B_setup()
    return {'A_x': _A_in['x'], 'A_wq': _A_in['wq'], 'A_wk': _A_in['wk'], 'A_wv': _A_in['wv'], 'A_wo': _A_in['wo'], 'A_beta': _A_in['beta'], 'B_x': _B_in['x'], 'B_w_r': _B_in['w_r'], 'B_w_gate': _B_in['w_gate'], 'B_w_up': _B_in['w_up'], 'B_w_down': _B_in['w_down']}

def reference(A_x, A_wq, A_wk, A_wv, A_wo, A_beta, B_x, B_w_r, B_w_gate, B_w_up, B_w_down):

    def _A_ref(x, wq, wk, wv, wo, beta):
        B, S, D = x.shape
        H = 32
        Dh = D // H
        N = 4
        L = S // N
        q = (lambda x, *d: x.transpose(*d))((x @ wq).reshape(B, S, H, Dh), 0, 2, 1, 3).reshape(B, H, N, L, Dh)
        k = (lambda x, *d: x.transpose(*d))((x @ wk).reshape(B, S, H, Dh), 0, 2, 1, 3).reshape(B, H, N, L, Dh)
        v = (lambda x, *d: x.transpose(*d))((x @ wv).reshape(B, S, H, Dh), 0, 2, 1, 3).reshape(B, H, N, L, Dh)
        phi = lambda t: jnp.where(t > 0, t + 1.0, jnp.exp(t))
        scale = Dh ** (-0.5)
        ar = jnp.arange(L)
        mask = (lambda x, dt: x.astype(dt))(ar[:, None] < ar[None, :], x.dtype) * -1000000000.0
        g = _sigmoid(beta).reshape(1, H, 1, 1)
        M = jnp.einsum('bhd,bhe->bhde', q[:, :, 0, 0, :] * 0.0, q[:, :, 0, 0, :] * 0.0)
        z = q[:, :, 0, 0, :] * 0.0
        outs = []
        for s in range(N):
            qs, ks, vs = (q[:, :, s].copy(), k[:, :, s].copy(), v[:, :, s].copy())
            logits = jnp.einsum('bhqd,bhkd->bhqk', qs, ks) * scale + mask
            p = _softmax(logits, axis=-1)
            a_dot = jnp.einsum('bhqk,bhkd->bhqd', p, vs)
            pq = phi(qs)
            num = jnp.einsum('bhld,bhde->bhle', pq, M)
            den = jnp.einsum('bhld,bhd->bhl', pq, z)[..., None] + 1e-06
            a_mem = num / den
            o = g * a_mem + (1.0 - g) * a_dot
            outs.append(o)
            pk = phi(ks)
            M = M + jnp.einsum('bhld,bhle->bhde', pk, vs)
            z = z + jnp.einsum('bhld->bhd', pk)
        o = (lambda x, *d: x.transpose(*d))(jnp.stack(outs, 2).reshape(B, H, S, Dh), 0, 2, 1, 3).reshape(B, S, D)
        return o @ wo

    def _B_ref(x, w_r, w_gate, w_up, w_down):
        B, S, D = x.shape
        C = 1
        r = x @ w_r
        idx = jnp.argsort(-r, axis=-1)[:, :C]
        idx_e = jnp.repeat(idx.reshape(B, C, 1), D, axis=2)
        x_sel = jnp.take_along_axis(x, idx_e, axis=1)
        g = _silu(x_sel @ w_gate)
        u = x_sel @ w_up
        y = g * u @ w_down
        r_sel = _sigmoid(jnp.take_along_axis(r, idx, axis=1))
        y = y * r_sel.reshape(B, C, 1)
        b_off = (jnp.arange(B) * S).reshape(B, 1)
        flat_idx = (idx + b_off).reshape(B * C)
        zero = (x * 0.0).reshape(B * S, D)
        upd = _scatter_add(zero, flat_idx, y.reshape(B * C, D), axis=0)
        return x + upd.reshape(B, S, D)
    x = A_x
    h = x + _A_ref(_layernorm(x, axis=-1), A_wq, A_wk, A_wv, A_wo, A_beta)
    h2 = h + _B_ref(_layernorm(h, axis=-1), B_w_r, B_w_gate, B_w_up, B_w_down)
    return h2
```

```python
import jax
import jax.numpy as jnp
from jax import lax
import jax.experimental.pallas as pl
import jax.experimental.pallas.tpu as pltpu

S = 2048
D = 576
H = 32
DH = 18
NSEG = 4
L = S // NSEG
F = 4608
HPG = 7
NG = 5
DP = 640
GW = HPG * DH
LOG2E = 1.4426950408889634
BF = jnp.bfloat16
F32 = jnp.float32
NEG = -1e30


def _nt(a, b):
    return lax.dot_general(a, b, (((1,), (1,)), ((), ())), preferred_element_type=F32)


def _nn(a, b):
    return jnp.dot(a, b, preferred_element_type=F32)


def _phi(t):
    return jnp.where(t > 0, t + 1.0, jnp.exp(jnp.minimum(t, 0.0)))


def _layernorm_cols(x):
    m = jnp.mean(x, axis=0, keepdims=True)
    d = x - m
    v = jnp.mean(d * d, axis=0, keepdims=True)
    return d * lax.rsqrt(v + 1e-5)


def _kernel(beta_ref, wr_ref,
            xT_hbm, wq_hbm, wk_hbm, wv_hbm, wo_hbm, wg_hbm, wu_hbm, wdT_hbm,
            outT_hbm,
            xT_v, wq_v, wk_v, wv_v, wo_v, wg_v, wu_v, wdT_v,
            wT, woT, gate_m, wr_m,
            xnT_s, k_s, qT_s, pqT_s, pkT_s, vT_s, oT_s,
            mt_s, maug_s,
            hnT_v, outT_v, r_v, tr_s,
            sem_in, sem_out):

    def cp_x(s):
        return pltpu.make_async_copy(xT_hbm.at[:, pl.ds(s * L, L)], xT_v.at[:, pl.ds(s * L, L)], sem_in.at[s])
    cp_wq = pltpu.make_async_copy(wq_hbm, wq_v, sem_in.at[4])
    cp_wk = pltpu.make_async_copy(wk_hbm, wk_v, sem_in.at[5])
    cp_wv = pltpu.make_async_copy(wv_hbm, wv_v, sem_in.at[6])
    cp_wo = pltpu.make_async_copy(wo_hbm, wo_v, sem_in.at[7])
    cp_wg = pltpu.make_async_copy(wg_hbm, wg_v, sem_in.at[8])
    cp_wu = pltpu.make_async_copy(wu_hbm, wu_v, sem_in.at[9])
    cp_wd = pltpu.make_async_copy(wdT_hbm, wdT_v, sem_in.at[10])
    cp_wq.start()
    cp_wk.start()
    cp_wv.start()
    for s in range(NSEG):
        cp_x(s).start()
    cp_wo.start()
    cp_wg.start()
    cp_wu.start()
    cp_wd.start()

    def cp_out(s):
        return pltpu.make_async_copy(outT_v.at[:, pl.ds(s * L, L)], outT_hbm.at[:, pl.ds(s * L, L)], sem_out.at[s])

    oT_s[...] = jnp.zeros(oT_s.shape, F32)
    mt_s[...] = jnp.zeros(mt_s.shape, F32)
    maug_s[...] = jnp.zeros(maug_s.shape, BF)
    xnT_s[D:DP, :] = jnp.zeros((DP - D, L), BF)
    zpad = jnp.zeros((48, L), BF)
    qT_s[4 * 128 + 80:5 * 128, :] = zpad
    pqT_s[4 * 128 + 80:5 * 128, :] = zpad
    pkT_s[4 * 128 + 80:5 * 128, :] = zpad
    vT_s[4 * 128 + 80:5 * 128, :] = zpad

    gate = jax.nn.sigmoid(beta_ref[...].astype(F32))
    rows = lax.broadcasted_iota(jnp.int32, (128, 128), 0)
    for g in range(NG):
        gm = jnp.zeros((128, 128), F32)
        for j in range(HPG):
            h = g * HPG + j
            if h < H:
                sel = (rows >= DH * j) & (rows < DH * (j + 1))
                gm = jnp.where(sel, jnp.broadcast_to(gate[:, h:h + 1], (128, 128)), gm)
        gate_m[g * 128:(g + 1) * 128, :] = gm

    wr_row = wr_ref[...].astype(F32)
    wr_row = jnp.concatenate([wr_row, jnp.zeros((1, DP - D), F32)], axis=1)
    for kb in range(DP // 128):
        wr_m[kb * 128:(kb + 1) * 128, :] = jnp.broadcast_to(wr_row[:, kb * 128:(kb + 1) * 128], (128, 128)).T

    def gap_block(w, g):
        if g < NG - 1:
            return w[:, GW * g:GW * g + 128]
        rem = D - GW * g
        return jnp.concatenate([w[:, GW * g:D], jnp.zeros((D, 128 - rem), BF)], axis=1)

    def transpose_store(w, base):
        for g in range(NG):
            blk = gap_block(w, g)
            blk = jnp.concatenate([blk, jnp.zeros((DP - D, 128), BF)], axis=0)
            for kb in range(DP // 128):
                wT[base + g * 128:base + (g + 1) * 128, kb * 128:(kb + 1) * 128] = (
                    blk[kb * 128:(kb + 1) * 128, :].T)

    cp_wq.wait()
    transpose_store(wq_v[...], 0)
    cp_wk.wait()
    transpose_store(wk_v[...], DP)
    cp_wv.wait()
    transpose_store(wv_v[...], 2 * DP)

    def relayout_wo():
        wo = wo_v[...].astype(F32)
        for g in range(NG):
            n = GW if g < NG - 1 else D - GW * g
            blk = wo[GW * g:GW * g + n, :]
            blk = jnp.concatenate([blk, jnp.zeros((128 - n, D), F32)], axis=0)
            blk = jnp.concatenate([blk, jnp.zeros((128, DP - D), F32)], axis=1).astype(BF)
            for kb in range(DP // 128):
                woT[kb * 128:(kb + 1) * 128, g * 128:(g + 1) * 128] = blk[:, kb * 128:(kb + 1) * 128].T

    rows128 = lax.broadcasted_iota(jnp.int32, (128, L), 0)

    def phase_proj(s):
        col0 = pl.multiple_of(s * L, L)
        for c in range(L // 128):
            xr = xT_v[:, pl.ds(col0 + c * 128, 128)].astype(F32)
            xnT_s[0:D, c * 128:(c + 1) * 128] = _layernorm_cols(xr).astype(BF)
        xn = xnT_s[...]
        for g in range(NG):
            nr = 128 if g < NG - 1 else 80
            r = slice(g * 128, g * 128 + nr)
            q = _nn(wT[g * 128:g * 128 + nr, :], xn)
            qT_s[r, :] = (q * (LOG2E * DH ** -0.5)).astype(BF)
            pqT_s[r, :] = _phi(q).astype(BF)
            k = _nn(wT[DP + g * 128:DP + g * 128 + nr, :], xn)
            pkT_s[r, :] = _phi(k).astype(BF)
            kb16 = k.astype(BF)
            if nr < 128:
                kb16 = jnp.concatenate([kb16, jnp.zeros((128 - nr, L), BF)], axis=0)
            for c in range(L // 128):
                k_s[c * 128:(c + 1) * 128, g * 128:(g + 1) * 128] = kb16[:, c * 128:(c + 1) * 128].T
            v = _nn(wT[2 * DP + g * 128:2 * DP + g * 128 + nr, :], xn)
            if nr == 128:
                v = jnp.where(rows128 >= GW, 1.0, v)
            vT_s[r, :] = v.astype(BF)
        vT_s[4 * 128 + 80:5 * 128, :] = jnp.ones((48, L), BF)

    ones_u32 = jnp.uint32(0x3F803F80)

    def head(g, j):
        base = pl.multiple_of(g * 128, 128)
        r0 = DH * j
        a = (r0 // 16) * 16
        o = r0 - a
        r1 = o + DH
        rows8 = lax.broadcasted_iota(jnp.int32, (8, 128), 0)
        rows32 = lax.broadcasted_iota(jnp.int32, (32, 128), 0)
        hrow = (rows32 >= o) & (rows32 < o + DH)
        tri = (lax.broadcasted_iota(jnp.int32, (128, 128), 0)
               <= lax.broadcasted_iota(jnp.int32, (128, 128), 1))
        gm = gate_m[pl.ds(base + a, 32), :]
        h_idx = g * HPG + j

        def vaug(kb):
            v = vT_s[pl.ds(base + a, 32), kb * 128:(kb + 1) * 128]
            vu = pltpu.bitcast(v, jnp.uint32)
            u = r1 // 2
            parts = []
            for t in range(2):
                p = vu[t * 8:(t + 1) * 8]
                if u // 8 == t:
                    p = jnp.where(rows8 == (u % 8), ones_u32, p)
                parts.append(p)
            return pltpu.bitcast(jnp.concatenate(parts, axis=0), BF)

        for qb in range(L // 128):
            lo, hi = r0 // 2, (r0 + DH) // 2
            t0, t1 = lo // 8, (hi - 1) // 8
            qt = qT_s[pl.ds(base + 16 * t0, 16 * (t1 - t0 + 1)), qb * 128:(qb + 1) * 128]
            qu = pltpu.bitcast(qt, jnp.uint32)
            parts = []
            for t in range(8):
                if t < t0 or t > t1:
                    parts.append(jnp.zeros((8, 128), jnp.uint32))
                else:
                    p = qu[(t - t0) * 8:(t - t0 + 1) * 8]
                    msk = (rows8 + 8 * t >= lo) & (rows8 + 8 * t < hi)
                    parts.append(jnp.where(msk, p, jnp.uint32(0)))
            qm = pltpu.bitcast(jnp.concatenate(parts, axis=0), BF)

            acc = None
            m = None
            for kb in range(qb, -1, -1):
                kt = k_s[kb * 128:(kb + 1) * 128, pl.ds(base, 128)]
                st = _nn(kt, qm)
                if kb == qb:
                    st = jnp.where(tri, st, NEG)
                mt = jnp.max(st, axis=0, keepdims=True)
                if m is None:
                    m = mt
                    p = jnp.exp2(st - m).astype(BF)
                    acc = _nn(vaug(kb), p)
                else:
                    m_new = jnp.maximum(m, mt)
                    alpha = jnp.exp2(m - m_new)
                    p = jnp.exp2(st - m_new).astype(BF)
                    acc = alpha * acc + _nn(vaug(kb), p)
                    m = m_new
            a_dot = acc / acc[r1:r1 + 1, :]
            nm = _nn(maug_s[h_idx], pqT_s[pl.ds(base, 128), qb * 128:(qb + 1) * 128])
            a_mem = nm / (nm[r1:r1 + 1, :] + 1e-6)
            val = gm * a_mem + (1.0 - gm) * a_dot
            old = oT_s[pl.ds(base + a, 32), qb * 128:(qb + 1) * 128]
            oT_s[pl.ds(base + a, 32), qb * 128:(qb + 1) * 128] = jnp.where(hrow, val, old)

    def phase_attn():
        def gbody(g, c):
            for j in range(HPG):
                head(g, j)
            return c
        lax.fori_loop(0, NG - 1, gbody, 0)
        for j in range(H - HPG * (NG - 1)):
            head(NG - 1, j)

    def phase_mem():
        lanes = lax.broadcasted_iota(jnp.int32, (32, 128), 1)
        rows32 = lax.broadcasted_iota(jnp.int32, (32, 128), 0)
        for g in range(NG):
            mt = mt_s[g] + _nt(vT_s[g * 128:(g + 1) * 128, :], pkT_s[g * 128:(g + 1) * 128, :])
            mt_s[g] = mt
            z = mt[127:128, :]
            for j in range(HPG):
                hh = g * HPG + j
                if hh >= H:
                    continue
                r0 = DH * j
                a = (r0 // 16) * 16
                o = r0 - a
                r1 = o + DH
                w = jnp.where((rows32 == r1) | (rows32 == r1 + 1),
                              jnp.broadcast_to(z, (32, 128)), mt[a:a + 32])
                w = jnp.where((lanes >= r0) & (lanes < r0 + DH), w, 0.0)
                maug_s[hh] = w.astype(BF)

    def phase_out(s):
        for c in range(L // 128):
            col0 = pl.multiple_of(s * L + c * 128, 128)
            ob = oT_s[:, c * 128:(c + 1) * 128].astype(BF)
            a = _nn(woT[0:D, :], ob)
            hb = (xT_v[:, pl.ds(col0, 128)].astype(F32) + a).astype(BF)
            hf = hb.astype(F32)
            hn = _layernorm_cols(hf).astype(BF)
            hnf = hn.astype(F32)
            r_v[:, pl.ds(col0, 128)] = jnp.sum(hnf * wr_m[0:D, :], axis=0, keepdims=True)
            hnT_v[:, pl.ds(col0, 128)] = hn
            outT_v[:, pl.ds(col0, 128)] = (hf + hnf).astype(BF)

    cp_wo.wait()
    relayout_wo()
    for s in range(NSEG):
        cp_x(s).wait()

    def seg_body(s, c):
        with jax.named_scope("proj"):
            phase_proj(s)
        with jax.named_scope("attn"):
            phase_attn()
        with jax.named_scope("mem"):
            phase_mem()
        with jax.named_scope("out"):
            phase_out(s)
        return c
    lax.fori_loop(0, NSEG, seg_body, 0)

    for s in range(NSEG):
        cp_out(s).start()

    with jax.named_scope("moe"):
        r = r_v[...]
        rmax_v = jnp.max(r, axis=1, keepdims=True)
        lidx = lax.broadcasted_iota(jnp.int32, (1, S), 1)
        idx = jnp.min(jnp.where(r == rmax_v, lidx, S - 1))
        cb = pl.multiple_of((idx // 128) * 128, 128)
        lane = idx - cb
        rb = pl.multiple_of((lane // 16) * 16, 16)
        hn_blk = hnT_v[:, pl.ds(cb, 128)]
        hn_blk = jnp.concatenate([hn_blk, jnp.zeros((DP - D, 128), BF)], axis=0)
        for kb in range(DP // 128):
            tr_s[:, kb * 128:(kb + 1) * 128] = hn_blk[kb * 128:(kb + 1) * 128, :].T
        xs = tr_s[pl.ds(rb, 16), 0:D]
        cp_wg.wait()
        gt = _nn(xs, wg_v[...])
        cp_wu.wait()
        ut = _nn(xs, wu_v[...])
        mid = (gt * jax.nn.sigmoid(gt) * ut).astype(BF)
        cp_wd.wait()
        y = _nt(mid, wdT_v[...])
        sel = lax.broadcasted_iota(jnp.int32, (16, D), 0) == (lane - rb)
        y = jnp.sum(jnp.where(sel, y, 0.0), axis=0, keepdims=True) * jax.nn.sigmoid(rmax_v)
        y = jnp.concatenate([y, jnp.zeros((1, DP - D), F32)], axis=1)
        yT = jnp.concatenate(
            [jnp.broadcast_to(y[:, kb * 128:(kb + 1) * 128], (128, 128)).T for kb in range(DP // 128)], axis=0)
        for s in range(NSEG):
            cp_out(s).wait()
        old = outT_v[:, pl.ds(cb, 128)].astype(F32)
        lsel = lax.broadcasted_iota(jnp.int32, (D, 128), 1) == lane
        outT_v[:, pl.ds(cb, 128)] = (old + jnp.where(lsel, yT[0:D], 0.0)).astype(BF)
        cp = pltpu.make_async_copy(outT_v.at[:, pl.ds(cb, 128)], outT_hbm.at[:, pl.ds(cb, 128)], sem_out.at[0])
        cp.start()
        cp.wait()


@jax.jit
def pallas_sequential_preLN__memory_aug_infini_attn__moe_arch_mod__prompt_kernel(
        A_x, A_wq, A_wk, A_wv, A_wo, A_beta, B_x, B_w_r, B_w_gate, B_w_up, B_w_down):
    del B_x
    xT = A_x.reshape(S, D).T
    hbm = pl.BlockSpec(memory_space=pltpu.HBM)
    vmem = pltpu.VMEM
    outT = pl.pallas_call(
        _kernel,
        out_shape=jax.ShapeDtypeStruct((D, S), BF),
        in_specs=[pl.BlockSpec(memory_space=pltpu.VMEM), pl.BlockSpec(memory_space=pltpu.VMEM)] + [hbm] * 8,
        out_specs=hbm,
        scratch_shapes=[
            vmem((D, S), BF), vmem((D, D), BF), vmem((D, D), BF), vmem((D, D), BF), vmem((D, D), BF),
            vmem((D, F), BF), vmem((D, F), BF), vmem((D, F), BF),
            vmem((3 * DP, DP), BF), vmem((DP, DP), BF), vmem((DP, 128), F32), vmem((DP, 128), F32),
            vmem((DP, L), BF), vmem((L, DP), BF), vmem((DP, L), BF), vmem((DP, L), BF), vmem((DP, L), BF),
            vmem((DP, L), BF), vmem((DP, L), F32),
            vmem((NG, 128, 128), F32), vmem((H, 32, 128), BF),
            vmem((D, S), BF), vmem((D, S), BF), vmem((1, S), F32), vmem((128, DP), BF),
            pltpu.SemaphoreType.DMA((11,)), pltpu.SemaphoreType.DMA((NSEG,)),
        ],
        compiler_params=pltpu.CompilerParams(vmem_limit_bytes=100 * 1024 * 1024),
        name="infini_moe",
    )(A_beta.reshape(1, H), B_w_r.reshape(1, D), xT, A_wq, A_wk, A_wv, A_wo, B_w_gate, B_w_up, B_w_down.T)
    return outT.T.reshape(1, S, D)
```

```python
import jax
import jax.numpy as jnp
from jax import lax
import jax.experimental.pallas as pl
import jax.experimental.pallas.tpu as pltpu

S = 2048
D = 576
H = 32
DH = 18
NSEG = 4
L = S // NSEG
F = 4608
HPG = 7
NG = 5
DP = 640
GW = HPG * DH
NQB = S // 128
LOG2E = 1.4426950408889634
BF = jnp.bfloat16
F32 = jnp.float32
U32 = jnp.uint32
NEG = -1e30
ONES2 = 0x3F803F80

TILE = {}
for _kb in range(4):
    for _qb in range(_kb, 4):
        TILE[(_kb, _qb)] = len(TILE)


def _nt(a, b):
    return lax.dot_general(a, b, (((1,), (1,)), ((), ())), preferred_element_type=F32)


def _nn(a, b):
    return jnp.dot(a, b, preferred_element_type=F32)


def _bf(x):
    return pltpu.bitcast(x, BF)


def _u32(x):
    return pltpu.bitcast(x, U32)


def _cat(xs, axis):
    return jnp.concatenate(xs, axis=axis) if len(xs) > 1 else xs[0]


def _phi(t):
    return jnp.where(t > 0, t + 1.0, jnp.exp(jnp.minimum(t, 0.0)))


def _layernorm_cols(x):
    m = jnp.mean(x, axis=0, keepdims=True)
    d = x - m
    v = jnp.mean(d * d, axis=0, keepdims=True)
    return d * lax.rsqrt(v + 1e-5)


class _Head:
    def __init__(self, h):
        self.h = h
        self.g = h // HPG
        self.j = h % HPG
        self.b = self.g * 128
        self.r0 = DH * self.j
        self.a = (self.r0 // 16) * 16
        self.o = self.r0 - self.a
        self.r1 = self.o + DH


def _kernel(beta_ref, wr_ref,
            xT_hbm, wq_hbm, wk_hbm, wv_hbm, wo_hbm, wg_hbm, wu_hbm, wdT_hbm,
            outT_hbm,
            xT_v, wq_v, wk_v, wv_v, wo_v, wg_v, wu_v, wdT_v,
            wT, woT, gate_m, wr_m,
            xnT_s, k_s, qT_s, pqT_s, pkT_s, vT_s, oT_s,
            mt_s, maug_s, s_scr, p_scr,
            hnT_v, outT_v, r_v, tr_s,
            sem_in, sem_out):

    def cp_x(s):
        return pltpu.make_async_copy(xT_hbm.at[:, pl.ds(s * L, L)], xT_v.at[:, pl.ds(s * L, L)], sem_in.at[s])
    cp_wq = pltpu.make_async_copy(wq_hbm, wq_v, sem_in.at[4])
    cp_wk = pltpu.make_async_copy(wk_hbm, wk_v, sem_in.at[5])
    cp_wv = pltpu.make_async_copy(wv_hbm, wv_v, sem_in.at[6])
    cp_wo = pltpu.make_async_copy(wo_hbm, wo_v, sem_in.at[7])
    cp_wg = pltpu.make_async_copy(wg_hbm, wg_v, sem_in.at[8])
    cp_wu = pltpu.make_async_copy(wu_hbm, wu_v, sem_in.at[9])
    cp_wd = pltpu.make_async_copy(wdT_hbm, wdT_v, sem_in.at[10])
    cp_wq.start()
    cp_x(0).start()
    cp_wk.start()
    cp_wv.start()
    for s in range(1, NSEG):
        cp_x(s).start()
    cp_wo.start()
    cp_wg.start()
    cp_wu.start()
    cp_wd.start()

    def cp_out(s):
        return pltpu.make_async_copy(outT_v.at[:, pl.ds(s * L, L)], outT_hbm.at[:, pl.ds(s * L, L)], sem_out.at[s])

    xnT_s[:, D:DP, :] = jnp.zeros((2, DP - D, L), BF)
    zpad = jnp.zeros((NQB, 48, 128), BF)
    qT_s[:, 4 * 128 + 80:5 * 128, :] = zpad
    pqT_s[:, 4 * 128 + 80:5 * 128, :] = zpad
    pkT_s[:, 4 * 128 + 80:5 * 128, :] = zpad
    vT_s[:, 4 * 128 + 80:5 * 128, :] = jnp.ones((NQB, 48, 128), BF)
    oT_s[...] = jnp.zeros(oT_s.shape, F32)
    maug_s[0:H] = jnp.zeros((H, 32, 128), BF)

    gate = jax.nn.sigmoid(beta_ref[...].astype(F32))
    rows = lax.broadcasted_iota(jnp.int32, (128, 128), 0)
    for g in range(NG):
        gm = jnp.zeros((128, 128), F32)
        for j in range(HPG):
            h = g * HPG + j
            if h < H:
                sel = (rows >= DH * j) & (rows < DH * (j + 1))
                gm = jnp.where(sel, jnp.broadcast_to(gate[:, h:h + 1], (128, 128)), gm)
        gate_m[g * 128:(g + 1) * 128, :] = gm

    wr_row = wr_ref[...].astype(F32)
    wr_row = jnp.concatenate([wr_row, jnp.zeros((1, DP - D), F32)], axis=1)
    for kb in range(DP // 128):
        wr_m[kb * 128:(kb + 1) * 128, :] = jnp.broadcast_to(wr_row[:, kb * 128:(kb + 1) * 128], (128, 128)).T

    def gap_block(w, g):
        if g < NG - 1:
            return w[:, GW * g:GW * g + 128]
        rem = D - GW * g
        return jnp.concatenate([w[:, GW * g:D], jnp.zeros((D, 128 - rem), BF)], axis=1)

    def transpose_store(w, base):
        for g in range(NG):
            blk = gap_block(w, g)
            blk = jnp.concatenate([blk, jnp.zeros((DP - D, 128), BF)], axis=0)
            for kb in range(DP // 128):
                wT[base + g * 128:base + (g + 1) * 128, kb * 128:(kb + 1) * 128] = (
                    blk[kb * 128:(kb + 1) * 128, :].T)

    def relayout_wo():
        wo = wo_v[...].astype(F32)
        for g in range(NG):
            n = GW if g < NG - 1 else D - GW * g
            blk = wo[GW * g:GW * g + n, :]
            blk = jnp.concatenate([blk, jnp.zeros((128 - n, D), F32)], axis=0)
            blk = jnp.concatenate([blk, jnp.zeros((128, DP - D), F32)], axis=1).astype(BF)
            for kb in range(DP // 128):
                woT[kb * 128:(kb + 1) * 128, g * 128:(g + 1) * 128] = blk[:, kb * 128:(kb + 1) * 128].T

    def ln1(s, slot):
        col0 = pl.multiple_of(s * L, L)
        for c in range(L // 128):
            xr = xT_v[:, pl.ds(col0 + c * 128, 128)].astype(F32)
            xnT_s[slot, 0:D, c * 128:(c + 1) * 128] = _layernorm_cols(xr).astype(BF)

    def proj(s, slot):
        xn = xnT_s[slot]
        rows128 = lax.broadcasted_iota(jnp.int32, (128, L), 0)
        for g in range(NG):
            nr = 128 if g < NG - 1 else 80
            r = slice(g * 128, g * 128 + nr)
            q = _nn(wT[g * 128:g * 128 + nr, :], xn)
            qs = (q * (LOG2E * DH ** -0.5)).astype(BF)
            pq = _phi(q).astype(BF)
            k = _nn(wT[DP + g * 128:DP + g * 128 + nr, :], xn)
            pk = _phi(k).astype(BF)
            kb16 = k.astype(BF)
            if nr < 128:
                kb16 = jnp.concatenate([kb16, jnp.zeros((128 - nr, L), BF)], axis=0)
            v = _nn(wT[2 * DP + g * 128:2 * DP + g * 128 + nr, :], xn)
            if nr == 128:
                v = jnp.where(rows128 >= GW, 1.0, v)
            v = v.astype(BF)
            for c in range(L // 128):
                t = s * 4 + c
                cs = slice(c * 128, (c + 1) * 128)
                qT_s[t, r, :] = qs[:, cs]
                pqT_s[t, r, :] = pq[:, cs]
                pkT_s[t, r, :] = pk[:, cs]
                vT_s[t, r, :] = v[:, cs]
                k_s[g, pl.ds(pl.multiple_of(t * 128, 128), 128), :] = kb16[:, cs].T

    cp_wq.wait()
    transpose_store(wq_v[...], 0)
    cp_x(0).wait()
    ln1(0, 0)
    cp_wk.wait()
    transpose_store(wk_v[...], DP)
    cp_wv.wait()
    transpose_store(wv_v[...], 2 * DP)
    for s in range(1, NSEG):
        cp_x(s).wait()

    with jax.named_scope("proj"):
        for s in range(NSEG):
            if s + 1 < NSEG:
                ln1(s + 1, (s + 1) % 2)
            proj(s, s % 2)

    with jax.named_scope("mem"):
        lanes = lax.broadcasted_iota(jnp.int32, (32, 128), 1)
        rows32 = lax.broadcasted_iota(jnp.int32, (32, 128), 0)
        for g in range(NG):
            mt = jnp.zeros((128, 128), F32)
            for s in range(NSEG - 1):
                vv = _cat([vT_s[4 * s + c, g * 128:(g + 1) * 128, :] for c in range(4)], 1)
                pp = _cat([pkT_s[4 * s + c, g * 128:(g + 1) * 128, :] for c in range(4)], 1)
                mt = mt + _nt(vv, pp)
                z = mt[127:128, :]
                for j in range(HPG):
                    if g * HPG + j >= H:
                        continue
                    hd = _Head(g * HPG + j)
                    w = jnp.where((rows32 == hd.r1) | (rows32 == hd.r1 + 1),
                                  jnp.broadcast_to(z, (32, 128)), mt[hd.a:hd.a + 32])
                    w = jnp.where((lanes >= hd.r0) & (lanes < hd.r0 + DH), w, 0.0)
                    maug_s[(s + 1) * H + hd.h] = w.astype(BF)

    def qm_tile(t0q, hd, qb):
        rows8 = lax.broadcasted_iota(jnp.int32, (8, 128), 0)
        lo, hi = hd.r0 // 2, (hd.r0 + DH) // 2
        t0, t1 = lo // 8, (hi - 1) // 8
        qu = _u32(qT_s[t0q + qb, hd.b + 16 * t0:hd.b + 16 * (t1 + 1), :])
        parts = []
        for t in range(8):
            if t < t0 or t > t1:
                parts.append(jnp.zeros((8, 128), U32))
            else:
                p = qu[(t - t0) * 8:(t - t0 + 1) * 8]
                msk = (rows8 + 8 * t >= lo) & (rows8 + 8 * t < hi)
                parts.append(jnp.where(msk, p, jnp.uint32(0)))
        return _bf(jnp.concatenate(parts, axis=0))

    def vaug(t0q, hd, kb):
        rows8 = lax.broadcasted_iota(jnp.int32, (8, 128), 0)
        vu = _u32(vT_s[t0q + kb, hd.b + hd.a:hd.b + hd.a + 32, :])
        u = hd.r1 // 2
        parts = []
        for t in range(2):
            p = vu[t * 8:(t + 1) * 8]
            if u // 8 == t:
                p = jnp.where(rows8 == (u % 8), jnp.uint32(ONES2), p)
            parts.append(p)
        return _bf(jnp.concatenate(parts, axis=0))

    def stage_a(t0q, hd, kb, slot, qms, mx):
        tri = (lax.broadcasted_iota(jnp.int32, (128, 128), 0)
               <= lax.broadcasted_iota(jnp.int32, (128, 128), 1))
        kt = k_s[hd.g, pl.ds(pl.multiple_of((t0q + kb) * 128, 128), 128), :]
        st = _nn(kt, _cat(qms[kb:], 1))
        for qb in range(kb, 4):
            t = st[:, (qb - kb) * 128:(qb - kb + 1) * 128]
            if qb == kb:
                t = jnp.where(tri, t, NEG)
            s_scr[slot, TILE[(kb, qb)]] = t
            pm = jnp.max(t.reshape(16, 8, 128), axis=0)
            mx[qb] = pm if mx[qb] is None else jnp.maximum(mx[qb], pm)

    def stage_e(qb, slot, mx):
        m = jnp.max(mx[qb], axis=0, keepdims=True)
        for kb in range(qb + 1):
            p_scr[slot, TILE[(kb, qb)]] = jnp.exp2(s_scr[slot, TILE[(kb, qb)]] - m).astype(BF)

    def stage_c(s, t0q, hd, qb, slot):
        p = _cat([p_scr[slot, TILE[(kb, qb)]] for kb in range(qb + 1)], 0)
        acc = _nn(_cat([vaug(t0q, hd, kb) for kb in range(qb + 1)], 1), p)
        rows32 = lax.broadcasted_iota(jnp.int32, (32, 128), 0)
        hrow = (rows32 >= hd.o) & (rows32 < hd.o + DH)
        gt = gate_m[hd.b + hd.r0:hd.b + hd.r0 + 1, :]
        nm = _nn(maug_s[s * H + hd.h], pqT_s[t0q + qb, hd.b:hd.b + 128, :])
        c_dot = (1.0 - gt) / acc[hd.r1:hd.r1 + 1, :]
        c_mem = gt / (nm[hd.r1:hd.r1 + 1, :] + 1e-6)
        val = acc * c_dot + nm * c_mem
        pltpu.store(oT_s.at[t0q + qb, hd.b + hd.a:hd.b + hd.a + 32, :], val, mask=hrow)

    def attn_segment(s, carry):
        t0q = s * 4
        mxs = {}
        for t in range(H + 2):
            ha, he, hc = t, t - 1, t - 2
            if ha < H:
                qms = [qm_tile(t0q, _Head(ha), qb) for qb in range(4)]
                mxs[ha] = [None] * 4
            for i in range(4):
                if ha < H:
                    stage_a(t0q, _Head(ha), i, ha % 2, qms, mxs[ha])
                if 0 <= he < H:
                    stage_e(3 - i, he % 2, mxs[he])
                if 0 <= hc < H:
                    stage_c(s, t0q, _Head(hc), 3 - i, hc % 2)
        return carry

    with jax.named_scope("attn"):
        lax.fori_loop(0, NSEG, attn_segment, 0)

    cp_wo.wait()
    relayout_wo()
    with jax.named_scope("out"):
        for s in range(NSEG):
            ob = _cat([oT_s[4 * s + c].astype(BF) for c in range(4)], 1)
            a = _nn(woT[0:D, :], ob)
            for c in range(4):
                cs = slice((4 * s + c) * 128, (4 * s + c + 1) * 128)
                hb = (xT_v[:, cs].astype(F32) + a[:, c * 128:(c + 1) * 128]).astype(BF)
                hf = hb.astype(F32)
                hn = _layernorm_cols(hf).astype(BF)
                hnf = hn.astype(F32)
                r_v[:, cs] = jnp.sum(hnf * wr_m[0:D, :], axis=0, keepdims=True)
                hnT_v[:, cs] = hn
                outT_v[:, cs] = (hf + hnf).astype(BF)
            cp_out(s).start()

    with jax.named_scope("moe"):
        r = r_v[...]
        rmax_v = jnp.max(r, axis=1, keepdims=True)
        lidx = lax.broadcasted_iota(jnp.int32, (1, S), 1)
        idx = jnp.min(jnp.where(r == rmax_v, lidx, S - 1))
        cb = pl.multiple_of((idx // 128) * 128, 128)
        lane = idx - cb
        rb = pl.multiple_of((lane // 16) * 16, 16)
        hn_blk = hnT_v[:, pl.ds(cb, 128)]
        hn_blk = jnp.concatenate([hn_blk, jnp.zeros((DP - D, 128), BF)], axis=0)
        for kb in range(DP // 128):
            tr_s[:, kb * 128:(kb + 1) * 128] = hn_blk[kb * 128:(kb + 1) * 128, :].T
        xs = tr_s[pl.ds(rb, 16), 0:D]
        cp_wg.wait()
        gt = _nn(xs, wg_v[...])
        cp_wu.wait()
        ut = _nn(xs, wu_v[...])
        mid = (gt * jax.nn.sigmoid(gt) * ut).astype(BF)
        cp_wd.wait()
        y = _nt(mid, wdT_v[...])
        sel = lax.broadcasted_iota(jnp.int32, (16, D), 0) == (lane - rb)
        y = jnp.sum(jnp.where(sel, y, 0.0), axis=0, keepdims=True) * jax.nn.sigmoid(rmax_v)
        y = jnp.concatenate([y, jnp.zeros((1, DP - D), F32)], axis=1)
        yT = jnp.concatenate(
            [jnp.broadcast_to(y[:, kb * 128:(kb + 1) * 128], (128, 128)).T for kb in range(DP // 128)], axis=0)
        for s in range(NSEG):
            cp_out(s).wait()
        old = outT_v[:, pl.ds(cb, 128)].astype(F32)
        lsel = lax.broadcasted_iota(jnp.int32, (D, 128), 1) == lane
        outT_v[:, pl.ds(cb, 128)] = (old + jnp.where(lsel, yT[0:D], 0.0)).astype(BF)
        cp = pltpu.make_async_copy(outT_v.at[:, pl.ds(cb, 128)], outT_hbm.at[:, pl.ds(cb, 128)], sem_out.at[0])
        cp.start()
        cp.wait()


@jax.jit
def pallas_sequential_preLN__memory_aug_infini_attn__moe_arch_mod__prompt_kernel(
        A_x, A_wq, A_wk, A_wv, A_wo, A_beta, B_x, B_w_r, B_w_gate, B_w_up, B_w_down):
    del B_x
    xT = A_x.reshape(S, D).T
    hbm = pl.BlockSpec(memory_space=pltpu.HBM)
    vmem = pltpu.VMEM
    outT = pl.pallas_call(
        _kernel,
        out_shape=jax.ShapeDtypeStruct((D, S), BF),
        in_specs=[pl.BlockSpec(memory_space=pltpu.VMEM), pl.BlockSpec(memory_space=pltpu.VMEM)] + [hbm] * 8,
        out_specs=hbm,
        scratch_shapes=[
            vmem((D, S), BF), vmem((D, D), BF), vmem((D, D), BF), vmem((D, D), BF), vmem((D, D), BF),
            vmem((D, F), BF), vmem((D, F), BF), vmem((D, F), BF),
            vmem((3 * DP, DP), BF), vmem((DP, DP), BF), vmem((DP, 128), F32), vmem((DP, 128), F32),
            vmem((2, DP, L), BF), vmem((NG, S, 128), BF),
            vmem((NQB, DP, 128), BF), vmem((NQB, DP, 128), BF), vmem((NQB, DP, 128), BF), vmem((NQB, DP, 128), BF),
            vmem((NQB, DP, 128), F32),
            vmem((NG, 128, 128), F32), vmem((NSEG * H, 32, 128), BF),
            vmem((2, 10, 128, 128), F32), vmem((2, 10, 128, 128), BF),
            vmem((D, S), BF), vmem((D, S), BF), vmem((1, S), F32), vmem((128, DP), BF),
            pltpu.SemaphoreType.DMA((11,)), pltpu.SemaphoreType.DMA((NSEG,)),
        ],
        compiler_params=pltpu.CompilerParams(vmem_limit_bytes=100 * 1024 * 1024),
        name="infini_moe",
    )(A_beta.reshape(1, H), B_w_r.reshape(1, D), xT, A_wq, A_wk, A_wv, A_wo, B_w_gate, B_w_up, B_w_down.T)
    return outT.T.reshape(1, S, D)
```

```python
import jax
import jax.numpy as jnp
from jax import lax
import jax.experimental.pallas as pl
import jax.experimental.pallas.tpu as pltpu

S = 2048
D = 576
H = 32
DH = 18
NSEG = 4
L = S // NSEG
F = 4608
HPG = 7
NG = 5
DP = 640
GW = HPG * DH
NQB = S // 128
LOG2E = 1.4426950408889634
BF = jnp.bfloat16
F32 = jnp.float32
U32 = jnp.uint32
NEG = -1e30
ONES2 = 0x3F803F80

TILE = {}
for _kb in range(4):
    for _qb in range(_kb, 4):
        TILE[(_kb, _qb)] = len(TILE)


def _nt(a, b):
    return lax.dot_general(a, b, (((1,), (1,)), ((), ())), preferred_element_type=F32)


def _nn(a, b):
    return jnp.dot(a, b, preferred_element_type=F32)


def _bf(x):
    return pltpu.bitcast(x, BF)


def _u32(x):
    return pltpu.bitcast(x, U32)


def _cat(xs, axis):
    return jnp.concatenate(xs, axis=axis) if len(xs) > 1 else xs[0]


def _phi(t):
    return jnp.where(t > 0, t + 1.0, jnp.exp(jnp.minimum(t, 0.0)))


def _layernorm_cols(x):
    m = jnp.mean(x, axis=0, keepdims=True)
    d = x - m
    v = jnp.mean(d * d, axis=0, keepdims=True)
    return d * lax.rsqrt(v + 1e-5)


class _Head:
    def __init__(self, h):
        self.h = h
        self.g = h // HPG
        self.j = h % HPG
        self.b = self.g * 128
        self.r0 = DH * self.j
        self.a = (self.r0 // 16) * 16
        self.o = self.r0 - self.a
        self.r1 = self.o + DH


def _kernel(beta_ref, wr_ref,
            xT_hbm, wq_hbm, wk_hbm, wv_hbm, wo_hbm, wg_hbm, wu_hbm, wdT_hbm,
            outT_hbm,
            xT_v, wq_v, wk_v, wv_v, wo_v, wg_v, wu_v, wdT_v,
            wT, woT, gate_m, wr_m,
            xnT_s, k_s, qT_s, pqT_s, pkT_s, vT_s, oT_s,
            mt_s, maug_s, s_scr, p_scr,
            hnT_v, outT_v, r_v, tr_s, h_s,
            sem_in, sem_out):

    def cp_x(s):
        return pltpu.make_async_copy(xT_hbm.at[:, pl.ds(s * L, L)], xT_v.at[:, pl.ds(s * L, L)], sem_in.at[s])
    cp_wq = pltpu.make_async_copy(wq_hbm, wq_v, sem_in.at[4])
    cp_wk = pltpu.make_async_copy(wk_hbm, wk_v, sem_in.at[5])
    cp_wv = pltpu.make_async_copy(wv_hbm, wv_v, sem_in.at[6])
    cp_wo = pltpu.make_async_copy(wo_hbm, wo_v, sem_in.at[7])
    cp_wg = pltpu.make_async_copy(wg_hbm, wg_v, sem_in.at[8])
    cp_wu = pltpu.make_async_copy(wu_hbm, wu_v, sem_in.at[9])
    cp_wd = pltpu.make_async_copy(wdT_hbm, wdT_v, sem_in.at[10])
    cp_x(0).start()
    cp_wq.start()
    cp_wk.start()
    cp_wv.start()
    for s in range(1, NSEG):
        cp_x(s).start()
    cp_wo.start()

    def cp_out(s):
        return pltpu.make_async_copy(outT_v.at[:, pl.ds(s * L, L)], outT_hbm.at[:, pl.ds(s * L, L)], sem_out.at[s])

    xnT_s[:, D:DP, :] = jnp.zeros((2, DP - D, L), BF)
    zpad = jnp.zeros((NQB, 48, 128), BF)
    qT_s[:, 4 * 128 + 80:5 * 128, :] = zpad
    pqT_s[:, 4 * 128 + 80:5 * 128, :] = zpad
    pkT_s[:, 4 * 128 + 80:5 * 128, :] = zpad
    vT_s[:, 4 * 128 + 80:5 * 128, :] = jnp.ones((NQB, 48, 128), BF)
    for g in range(NG - 1):
        oT_s[:, g * 128 + 120:(g + 1) * 128, :] = jnp.zeros((NQB, 8, 128), F32)
    oT_s[:, 4 * 128 + 64:5 * 128, :] = jnp.zeros((NQB, 64, 128), F32)
    maug_s[0:H] = jnp.zeros((H, 32, 128), BF)

    gate = jax.nn.sigmoid(beta_ref[...].astype(F32))
    rows = lax.broadcasted_iota(jnp.int32, (128, 128), 0)
    for g in range(NG):
        gm = jnp.zeros((128, 128), F32)
        for j in range(HPG):
            h = g * HPG + j
            if h < H:
                sel = (rows >= DH * j) & (rows < DH * (j + 1))
                gm = jnp.where(sel, jnp.broadcast_to(gate[:, h:h + 1], (128, 128)), gm)
        gate_m[g * 128:(g + 1) * 128, :] = gm

    wr_row = wr_ref[...].astype(F32)
    wr_row = jnp.concatenate([wr_row, jnp.zeros((1, DP - D), F32)], axis=1)
    for kb in range(DP // 128):
        wr_m[kb * 128:(kb + 1) * 128, :] = jnp.broadcast_to(wr_row[:, kb * 128:(kb + 1) * 128], (128, 128)).T

    def gap_block(w, g):
        c0 = (GW * g // 128) * 128
        c1 = min(c0 + 256, D)
        w = w[:, c0:c1]
        if g < NG - 1:
            return w[:, GW * g - c0:GW * g - c0 + 128]
        rem = D - GW * g
        return jnp.concatenate([w[:, GW * g - c0:], jnp.zeros((D, 128 - rem), BF)], axis=1)

    def transpose_store(w_ref, base, g):
        blk = gap_block(w_ref, g)
        blk = jnp.concatenate([blk, jnp.zeros((DP - D, 128), BF)], axis=0)
        for kb in range(DP // 128):
            wT[base + g * 128:base + (g + 1) * 128, kb * 128:(kb + 1) * 128] = (
                blk[kb * 128:(kb + 1) * 128, :].T)

    def relayout_wo(g):
        n = GW if g < NG - 1 else D - GW * g
        a0 = (GW * g // 16) * 16
        a1 = min(a0 + 144, D)
        wo = wo_v[a0:a1, :].astype(F32)
        blk = wo[GW * g - a0:GW * g - a0 + n, :]
        blk = jnp.concatenate([blk, jnp.zeros((128 - n, D), F32)], axis=0)
        blk = jnp.concatenate([blk, jnp.zeros((128, DP - D), F32)], axis=1).astype(BF)
        for kb in range(DP // 128):
            woT[kb * 128:(kb + 1) * 128, g * 128:(g + 1) * 128] = blk[:, kb * 128:(kb + 1) * 128].T

    def ln1(s, slot, c):
        xr = xT_v[:, s * L + c * 128:s * L + (c + 1) * 128].astype(F32)
        xnT_s[slot, 0:D, c * 128:(c + 1) * 128] = _layernorm_cols(xr).astype(BF)

    def proj(s, slot, first, fillers):
        xn = xnT_s[slot]
        rows128 = lax.broadcasted_iota(jnp.int32, (128, L), 0)

        def tiles(g):
            nr = 128 if g < NG - 1 else 80
            return nr, slice(g * 128, g * 128 + nr)

        def do_q(g):
            nr, r = tiles(g)
            q = _nn(wT[g * 128:g * 128 + nr, :], xn)
            qs = (q * (LOG2E * DH ** -0.5)).astype(BF)
            pq = _phi(q).astype(BF)
            for c in range(L // 128):
                cs = slice(c * 128, (c + 1) * 128)
                qT_s[s * 4 + c, r, :] = qs[:, cs]
                pqT_s[s * 4 + c, r, :] = pq[:, cs]

        def do_k(g):
            nr, r = tiles(g)
            k = _nn(wT[DP + g * 128:DP + g * 128 + nr, :], xn)
            pk = _phi(k).astype(BF)
            kb16 = k.astype(BF)
            if nr < 128:
                kb16 = jnp.concatenate([kb16, jnp.zeros((128 - nr, L), BF)], axis=0)
            for c in range(L // 128):
                cs = slice(c * 128, (c + 1) * 128)
                pkT_s[s * 4 + c, r, :] = pk[:, cs]
                k_s[g, (s * 4 + c) * 128:(s * 4 + c + 1) * 128, :] = kb16[:, cs].T

        def do_v(g):
            nr, r = tiles(g)
            v = _nn(wT[2 * DP + g * 128:2 * DP + g * 128 + nr, :], xn)
            if nr == 128:
                v = jnp.where(rows128 >= GW, 1.0, v)
            v = v.astype(BF)
            for c in range(L // 128):
                vT_s[s * 4 + c, r, :] = v[:, c * 128:(c + 1) * 128]

        for fn, cp, w_ref, base in ((do_q, cp_wq, wq_v, 0), (do_k, cp_wk, wk_v, DP), (do_v, cp_wv, wv_v, 2 * DP)):
            if first:
                cp.wait()
            for g in range(NG):
                if first:
                    transpose_store(w_ref, base, g)
                fn(g)
                f = fillers.get((base // DP) * NG + g)
                if f is not None:
                    f()

    cp_x(0).wait()
    for c in range(4):
        ln1(0, 0, c)
    with jax.named_scope("proj"):
        for s in range(NSEG):
            fillers = {}
            if s + 1 < NSEG:
                fillers[9] = lambda s=s: cp_x(s + 1).wait()
                for c in range(4):
                    fillers[10 + c] = lambda s=s, c=c: ln1(s + 1, (s + 1) % 2, c)
            if s == 0:
                fillers[14] = lambda: (cp_wg.start(), cp_wu.start(), cp_wd.start())
            if s == 1:
                fillers[0] = lambda: cp_wo.wait()
                for g in range(NG):
                    fillers[1 + g] = lambda g=g: relayout_wo(g)
            proj(s, s % 2, s == 0, fillers)

    with jax.named_scope("mem"):
        lanes = lax.broadcasted_iota(jnp.int32, (32, 128), 1)
        rows32 = lax.broadcasted_iota(jnp.int32, (32, 128), 0)
        for g in range(NG):
            mt = jnp.zeros((128, 128), F32)
            for s in range(NSEG - 1):
                vv = _cat([vT_s[4 * s + c, g * 128:(g + 1) * 128, :] for c in range(4)], 1)
                pp = _cat([pkT_s[4 * s + c, g * 128:(g + 1) * 128, :] for c in range(4)], 1)
                mt = mt + _nt(vv, pp)
                z = mt[127:128, :]
                for j in range(HPG):
                    if g * HPG + j >= H:
                        continue
                    hd = _Head(g * HPG + j)
                    w = jnp.where((rows32 == hd.r1) | (rows32 == hd.r1 + 1),
                                  jnp.broadcast_to(z, (32, 128)), mt[hd.a:hd.a + 32])
                    w = jnp.where((lanes >= hd.r0) & (lanes < hd.r0 + DH), w, 0.0)
                    maug_s[(s + 1) * H + hd.h] = w.astype(BF)

    def qm_tile(t0q, hd, qb):
        rows8 = lax.broadcasted_iota(jnp.int32, (8, 128), 0)
        lo, hi = hd.r0 // 2, (hd.r0 + DH) // 2
        t0, t1 = lo // 8, (hi - 1) // 8
        qu = _u32(qT_s[t0q + qb, hd.b + 16 * t0:hd.b + 16 * (t1 + 1), :])
        parts = []
        for t in range(8):
            if t < t0 or t > t1:
                parts.append(jnp.zeros((8, 128), U32))
            else:
                p = qu[(t - t0) * 8:(t - t0 + 1) * 8]
                msk = (rows8 + 8 * t >= lo) & (rows8 + 8 * t < hi)
                parts.append(jnp.where(msk, p, jnp.uint32(0)))
        return _bf(jnp.concatenate(parts, axis=0))

    def vaug(t0q, hd, kb):
        rows8 = lax.broadcasted_iota(jnp.int32, (8, 128), 0)
        vu = _u32(vT_s[t0q + kb, hd.b + hd.a:hd.b + hd.a + 32, :])
        u = hd.r1 // 2
        parts = []
        for t in range(2):
            p = vu[t * 8:(t + 1) * 8]
            if u // 8 == t:
                p = jnp.where(rows8 == (u % 8), jnp.uint32(ONES2), p)
            parts.append(p)
        return _bf(jnp.concatenate(parts, axis=0))

    def stage_a(t0q, hd, kb, slot, qms, mx):
        tri = (lax.broadcasted_iota(jnp.int32, (128, 128), 0)
               <= lax.broadcasted_iota(jnp.int32, (128, 128), 1))
        kt = k_s[hd.g, pl.ds(pl.multiple_of((t0q + kb) * 128, 128), 128), :]
        st = _nn(kt, _cat(qms[kb:], 1))
        for qb in range(kb, 4):
            t = st[:, (qb - kb) * 128:(qb - kb + 1) * 128]
            if qb == kb:
                t = jnp.where(tri, t, NEG)
            s_scr[slot, TILE[(kb, qb)]] = t
            pm = jnp.max(t.reshape(16, 8, 128), axis=0)
            mx[qb] = pm if mx[qb] is None else jnp.maximum(mx[qb], pm)

    def stage_e(qb, slot, mx):
        m = jnp.max(mx[qb], axis=0, keepdims=True)
        for kb in range(qb + 1):
            p_scr[slot, TILE[(kb, qb)]] = jnp.exp2(s_scr[slot, TILE[(kb, qb)]] - m).astype(BF)

    def stage_c(s, t0q, hd, qb, slot):
        p = _cat([p_scr[slot, TILE[(kb, qb)]] for kb in range(qb + 1)], 0)
        acc = _nn(_cat([vaug(t0q, hd, kb) for kb in range(qb + 1)], 1), p)
        rows32 = lax.broadcasted_iota(jnp.int32, (32, 128), 0)
        hrow = (rows32 >= hd.o) & (rows32 < hd.o + DH)
        gt = gate_m[hd.b + hd.r0:hd.b + hd.r0 + 1, :]
        nm = _nn(maug_s[s * H + hd.h], pqT_s[t0q + qb, hd.b:hd.b + 128, :])
        c_dot = (1.0 - gt) / acc[hd.r1:hd.r1 + 1, :]
        c_mem = gt / (nm[hd.r1:hd.r1 + 1, :] + 1e-6)
        val = acc * c_dot + nm * c_mem
        pltpu.store(oT_s.at[t0q + qb, hd.b + hd.a:hd.b + hd.a + 32, :], val, mask=hrow)

    def attn_segment(s, carry):
        t0q = s * 4
        mxs = {}
        for t in range(H + 2):
            ha, he, hc = t, t - 1, t - 2
            if ha < H:
                qms = [qm_tile(t0q, _Head(ha), qb) for qb in range(4)]
                mxs[ha] = [None] * 4
            for i in range(4):
                if ha < H:
                    stage_a(t0q, _Head(ha), i, ha % 2, qms, mxs[ha])
                if 0 <= he < H:
                    stage_e(i, he % 2, mxs[he])
                if 0 <= hc < H:
                    stage_c(s, t0q, _Head(hc), i, hc % 2)
        return carry

    with jax.named_scope("attn"):
        lax.fori_loop(0, NSEG, attn_segment, 0)

    def out_ln(s, c):
        col = pl.multiple_of((4 * s + c) * 128, 128)
        cs = pl.ds(col, 128)
        hf = h_s[s % 2, c].astype(F32)
        hn = _layernorm_cols(hf).astype(BF)
        hnf = hn.astype(F32)
        r_v[:, cs] = jnp.sum(hnf * wr_m[0:D, :], axis=0, keepdims=True)
        hnT_v[:, cs] = hn
        outT_v[:, cs] = (hf + hnf).astype(BF)

    def out_mm(s, fillers):
        ob = _cat([oT_s[4 * s + c].astype(BF) for c in range(4)], 1)
        for i, (r0, r1) in enumerate(((0, 128), (128, 256), (256, 384), (384, 512), (512, D))):
            a = _nn(woT[r0:r1, :], ob)
            hb = (xT_v[r0:r1, pl.ds(pl.multiple_of(s * L, L), L)].astype(F32) + a).astype(BF)
            for c in range(4):
                h_s[s % 2, c, r0:r1, :] = hb[:, c * 128:(c + 1) * 128]
            if i < len(fillers):
                fillers[i]()

    with jax.named_scope("out"):
        out_mm(0, [])

        def out_body(s, carry):
            out_mm(s + 1, [lambda c=c: out_ln(s, c) for c in range(4)])
            col = pl.multiple_of(s * L, L)
            pltpu.make_async_copy(outT_v.at[:, pl.ds(col, L)], outT_hbm.at[:, pl.ds(col, L)], sem_out.at[s]).start()
            return carry
        lax.fori_loop(0, NSEG - 1, out_body, 0)
        for c in range(4):
            out_ln(NSEG - 1, c)
        cp_out(NSEG - 1).start()

    with jax.named_scope("moe"):
        r = r_v[...]
        rmax_v = jnp.max(r, axis=1, keepdims=True)
        lidx = lax.broadcasted_iota(jnp.int32, (1, S), 1)
        idx = jnp.min(jnp.where(r == rmax_v, lidx, S - 1))
        cb = pl.multiple_of((idx // 128) * 128, 128)
        lane = idx - cb
        rb = pl.multiple_of((lane // 16) * 16, 16)
        hn_blk = hnT_v[:, pl.ds(cb, 128)]
        hn_blk = jnp.concatenate([hn_blk, jnp.zeros((DP - D, 128), BF)], axis=0)
        for kb in range(DP // 128):
            tr_s[:, kb * 128:(kb + 1) * 128] = hn_blk[kb * 128:(kb + 1) * 128, :].T
        xs = tr_s[pl.ds(rb, 16), 0:D]
        cp_wg.wait()
        gt = _nn(xs, wg_v[...])
        cp_wu.wait()
        ut = _nn(xs, wu_v[...])
        mid = (gt * jax.nn.sigmoid(gt) * ut).astype(BF)
        cp_wd.wait()
        y = _nt(mid, wdT_v[...])
        sel = lax.broadcasted_iota(jnp.int32, (16, D), 0) == (lane - rb)
        y = jnp.sum(jnp.where(sel, y, 0.0), axis=0, keepdims=True) * jax.nn.sigmoid(rmax_v)
        y = jnp.concatenate([y, jnp.zeros((1, DP - D), F32)], axis=1)
        yT = jnp.concatenate(
            [jnp.broadcast_to(y[:, kb * 128:(kb + 1) * 128], (128, 128)).T for kb in range(DP // 128)], axis=0)
        for s in range(NSEG):
            cp_out(s).wait()
        old = outT_v[:, pl.ds(cb, 128)].astype(F32)
        lsel = lax.broadcasted_iota(jnp.int32, (D, 128), 1) == lane
        outT_v[:, pl.ds(cb, 128)] = (old + jnp.where(lsel, yT[0:D], 0.0)).astype(BF)
        cp = pltpu.make_async_copy(outT_v.at[:, pl.ds(cb, 128)], outT_hbm.at[:, pl.ds(cb, 128)], sem_out.at[0])
        cp.start()
        cp.wait()


@jax.jit
def pallas_sequential_preLN__memory_aug_infini_attn__moe_arch_mod__prompt_kernel(
        A_x, A_wq, A_wk, A_wv, A_wo, A_beta, B_x, B_w_r, B_w_gate, B_w_up, B_w_down):
    del B_x
    xT = A_x.reshape(S, D).T
    hbm = pl.BlockSpec(memory_space=pltpu.HBM)
    vmem = pltpu.VMEM
    outT = pl.pallas_call(
        _kernel,
        out_shape=jax.ShapeDtypeStruct((D, S), BF),
        in_specs=[pl.BlockSpec(memory_space=pltpu.VMEM), pl.BlockSpec(memory_space=pltpu.VMEM)] + [hbm] * 8,
        out_specs=hbm,
        scratch_shapes=[
            vmem((D, S), BF), vmem((D, D), BF), vmem((D, D), BF), vmem((D, D), BF), vmem((D, D), BF),
            vmem((D, F), BF), vmem((D, F), BF), vmem((D, F), BF),
            vmem((3 * DP, DP), BF), vmem((DP, DP), BF), vmem((DP, 128), F32), vmem((DP, 128), F32),
            vmem((2, DP, L), BF), vmem((NG, S, 128), BF),
            vmem((NQB, DP, 128), BF), vmem((NQB, DP, 128), BF), vmem((NQB, DP, 128), BF), vmem((NQB, DP, 128), BF),
            vmem((NQB, DP, 128), F32),
            vmem((NG, 128, 128), F32), vmem((NSEG * H, 32, 128), BF),
            vmem((2, 10, 128, 128), F32), vmem((2, 10, 128, 128), BF),
            vmem((D, S), BF), vmem((D, S), BF), vmem((1, S), F32), vmem((128, DP), BF), vmem((2, 4, D, 128), BF),
            pltpu.SemaphoreType.DMA((11,)), pltpu.SemaphoreType.DMA((NSEG,)),
        ],
        compiler_params=pltpu.CompilerParams(vmem_limit_bytes=100 * 1024 * 1024),
        name="infini_moe",
    )(A_beta.reshape(1, H), B_w_r.reshape(1, D), xT, A_wq, A_wk, A_wv, A_wo, B_w_gate, B_w_up, B_w_down.T)
    return outT.T.reshape(1, S, D)
```

```python
import jax
import jax.numpy as jnp
from jax import lax
import jax.experimental.pallas as pl
import jax.experimental.pallas.tpu as pltpu

S = 2048
D = 576
H = 32
DH = 18
NSEG = 4
L = S // NSEG
F = 4608
HPG = 7
NG = 5
DP = 640
GW = HPG * DH
NQB = S // 128
LOG2E = 1.4426950408889634
BF = jnp.bfloat16
F32 = jnp.float32
U32 = jnp.uint32
NEG = -1e30
ONES2 = 0x3F803F80

TILE = {}
for _kb in range(4):
    for _qb in range(_kb, 4):
        TILE[(_kb, _qb)] = len(TILE)


def _nt(a, b):
    return lax.dot_general(a, b, (((1,), (1,)), ((), ())), preferred_element_type=F32)


def _nn(a, b):
    return jnp.dot(a, b, preferred_element_type=F32)


def _bf(x):
    return pltpu.bitcast(x, BF)


def _u32(x):
    return pltpu.bitcast(x, U32)


def _cat(xs, axis):
    return jnp.concatenate(xs, axis=axis) if len(xs) > 1 else xs[0]


def _phi(t):
    return jnp.where(t > 0, t + 1.0, jnp.exp(jnp.minimum(t, 0.0)))


def _layernorm_cols(x):
    m = jnp.mean(x, axis=0, keepdims=True)
    d = x - m
    v = jnp.mean(d * d, axis=0, keepdims=True)
    return d * lax.rsqrt(v + 1e-5)


class _Head:
    def __init__(self, h):
        self.h = h
        self.g = h // HPG
        self.j = h % HPG
        self.b = self.g * 128
        self.r0 = DH * self.j
        self.a = (self.r0 // 16) * 16
        self.o = self.r0 - self.a
        self.r1 = self.o + DH


def _kernel(beta_ref, wr_ref,
            xT_hbm, wq_hbm, wk_hbm, wv_hbm, wo_hbm, wg_hbm, wu_hbm, wdT_hbm,
            outT_hbm,
            xT_v, wq_v, wk_v, wv_v, wo_v, wg_v, wu_v, wdT_v,
            wT, woT, gate_m, wr_m,
            xnT_s, k_s, qT_s, pqT_s, pkT_s, vT_s, oT_s,
            nm_s, maug_s, s_scr, p_scr,
            hnT_v, outT_v, r_v, tr_s, h_s,
            sem_in, sem_out):

    def cp_x(s):
        return pltpu.make_async_copy(xT_hbm.at[:, pl.ds(s * L, L)], xT_v.at[:, pl.ds(s * L, L)], sem_in.at[s])
    cp_wq = pltpu.make_async_copy(wq_hbm, wq_v, sem_in.at[4])
    cp_wk = pltpu.make_async_copy(wk_hbm, wk_v, sem_in.at[5])
    cp_wv = pltpu.make_async_copy(wv_hbm, wv_v, sem_in.at[6])
    cp_wo = pltpu.make_async_copy(wo_hbm, wo_v, sem_in.at[7])
    cp_wg = pltpu.make_async_copy(wg_hbm, wg_v, sem_in.at[8])
    cp_wu = pltpu.make_async_copy(wu_hbm, wu_v, sem_in.at[9])
    cp_wd = pltpu.make_async_copy(wdT_hbm, wdT_v, sem_in.at[10])
    cp_x(0).start()
    cp_wq.start()
    cp_wk.start()
    cp_wv.start()
    for s in range(1, NSEG):
        cp_x(s).start()
    cp_wo.start()

    def cp_out(s):
        return pltpu.make_async_copy(outT_v.at[:, pl.ds(s * L, L)], outT_hbm.at[:, pl.ds(s * L, L)], sem_out.at[s])

    xnT_s[:, D:DP, :] = jnp.zeros((2, DP - D, L), BF)
    zpad = jnp.zeros((NQB, 48, 128), BF)
    qT_s[:, 4 * 128 + 80:5 * 128, :] = zpad
    pqT_s[:, 4 * 128 + 80:5 * 128, :] = zpad
    pkT_s[:, 4 * 128 + 80:5 * 128, :] = zpad
    vT_s[:, 4 * 128 + 80:5 * 128, :] = jnp.ones((NQB, 48, 128), BF)
    for g in range(NG - 1):
        oT_s[:, g * 128 + 120:(g + 1) * 128, :] = jnp.zeros((NQB, 8, 128), F32)
    oT_s[:, 4 * 128 + 64:5 * 128, :] = jnp.zeros((NQB, 64, 128), F32)
    maug_s[0:NG] = jnp.zeros((NG, 144, 128), BF)

    gate = jax.nn.sigmoid(beta_ref[...].astype(F32))
    rows = lax.broadcasted_iota(jnp.int32, (128, 128), 0)
    for g in range(NG):
        gm = jnp.zeros((128, 128), F32)
        for j in range(HPG):
            h = g * HPG + j
            if h < H:
                sel = (rows >= DH * j) & (rows < DH * (j + 1))
                gm = jnp.where(sel, jnp.broadcast_to(gate[:, h:h + 1], (128, 128)), gm)
        gate_m[g * 128:(g + 1) * 128, :] = gm

    wr_row = wr_ref[...].astype(F32)
    wr_row = jnp.concatenate([wr_row, jnp.zeros((1, DP - D), F32)], axis=1)
    for kb in range(DP // 128):
        wr_m[kb * 128:(kb + 1) * 128, :] = jnp.broadcast_to(wr_row[:, kb * 128:(kb + 1) * 128], (128, 128)).T

    def gap_block(w, g):
        c0 = (GW * g // 128) * 128
        c1 = min(c0 + 256, D)
        w = w[:, c0:c1]
        if g < NG - 1:
            return w[:, GW * g - c0:GW * g - c0 + 128]
        rem = D - GW * g
        return jnp.concatenate([w[:, GW * g - c0:], jnp.zeros((D, 128 - rem), BF)], axis=1)

    def transpose_store(w_ref, base, g):
        blk = gap_block(w_ref, g)
        blk = jnp.concatenate([blk, jnp.zeros((DP - D, 128), BF)], axis=0)
        for kb in range(DP // 128):
            wT[base + g * 128:base + (g + 1) * 128, kb * 128:(kb + 1) * 128] = (
                blk[kb * 128:(kb + 1) * 128, :].T)

    def relayout_wo(g):
        n = GW if g < NG - 1 else D - GW * g
        a0 = (GW * g // 16) * 16
        a1 = min(a0 + 144, D)
        wo = wo_v[a0:a1, :].astype(F32)
        blk = wo[GW * g - a0:GW * g - a0 + n, :]
        blk = jnp.concatenate([blk, jnp.zeros((128 - n, D), F32)], axis=0)
        blk = jnp.concatenate([blk, jnp.zeros((128, DP - D), F32)], axis=1).astype(BF)
        for kb in range(DP // 128):
            woT[kb * 128:(kb + 1) * 128, g * 128:(g + 1) * 128] = blk[:, kb * 128:(kb + 1) * 128].T

    def ln1(s, slot, c):
        xr = xT_v[:, pl.ds(pl.multiple_of(s * L + c * 128, 128), 128)].astype(F32)
        xnT_s[slot, 0:D, c * 128:(c + 1) * 128] = _layernorm_cols(xr).astype(BF)

    def proj(s, slot, first, fillers):
        xn = xnT_s[slot]
        rows128 = lax.broadcasted_iota(jnp.int32, (128, L), 0)

        def tiles(g):
            nr = 128 if g < NG - 1 else 80
            return nr, slice(g * 128, g * 128 + nr)

        def do_q(g):
            nr, r = tiles(g)
            q = _nn(wT[g * 128:g * 128 + nr, :], xn)
            qs = (q * (LOG2E * DH ** -0.5)).astype(BF)
            pq = _phi(q).astype(BF)
            for c in range(L // 128):
                cs = slice(c * 128, (c + 1) * 128)
                qT_s[s * 4 + c, r, :] = qs[:, cs]
                pqT_s[s * 4 + c, r, :] = pq[:, cs]

        def do_k(g):
            nr, r = tiles(g)
            k = _nn(wT[DP + g * 128:DP + g * 128 + nr, :], xn)
            pk = _phi(k).astype(BF)
            kb16 = k.astype(BF)
            if nr < 128:
                kb16 = jnp.concatenate([kb16, jnp.zeros((128 - nr, L), BF)], axis=0)
            for c in range(L // 128):
                cs = slice(c * 128, (c + 1) * 128)
                pkT_s[s * 4 + c, r, :] = pk[:, cs]
                k_s[g, pl.ds(pl.multiple_of((s * 4 + c) * 128, 128), 128), :] = kb16[:, cs].T

        def do_v(g):
            nr, r = tiles(g)
            v = _nn(wT[2 * DP + g * 128:2 * DP + g * 128 + nr, :], xn)
            if nr == 128:
                v = jnp.where(rows128 >= GW, 1.0, v)
            v = v.astype(BF)
            for c in range(L // 128):
                vT_s[s * 4 + c, r, :] = v[:, c * 128:(c + 1) * 128]

        for fn, cp, w_ref, base in ((do_q, cp_wq, wq_v, 0), (do_k, cp_wk, wk_v, DP), (do_v, cp_wv, wv_v, 2 * DP)):
            if first:
                cp.wait()
            for g in range(NG):
                if first:
                    transpose_store(w_ref, base, g)
                fn(g)
                f = fillers.get((base // DP) * NG + g)
                if f is not None:
                    f()

    cp_x(0).wait()
    for c in range(4):
        ln1(0, 0, c)
    with jax.named_scope("proj"):
        fillers = {9: lambda: [cp_x(i).wait() for i in range(1, NSEG)]}
        for c in range(4):
            fillers[10 + c] = lambda c=c: ln1(1, 1, c)
        fillers[14] = lambda: (cp_wg.start(), cp_wu.start(), cp_wd.start())
        proj(0, 0, True, fillers)
        cp_wo.wait()

        def proj_body(s, carry):
            nxt = jnp.minimum(s + 1, NSEG - 1)
            fl = {}
            for c in range(4):
                fl[8 + c] = lambda c=c: ln1(nxt, 1 - s % 2, c)
            proj(s, s % 2, False, fl)
            return carry
        lax.fori_loop(1, NSEG, proj_body, 0)
        for g in range(NG):
            relayout_wo(g)

    with jax.named_scope("mem"):
        rr = lax.broadcasted_iota(jnp.int32, (128, 128), 0)
        ll = lax.broadcasted_iota(jnp.int32, (128, 128), 1)
        same = jnp.zeros((128, 128), jnp.bool_)
        zsel = jnp.zeros((16, 128), jnp.bool_)
        r16 = lax.broadcasted_iota(jnp.int32, (16, 128), 0)
        l16 = lax.broadcasted_iota(jnp.int32, (16, 128), 1)
        for j in range(HPG):
            lo, hi = DH * j, DH * (j + 1)
            same = same | ((rr >= lo) & (rr < hi) & (ll >= lo) & (ll < hi))
            zsel = zsel | ((r16 == j) & (l16 >= lo) & (l16 < hi))
        for g in range(NG):
            mt = jnp.zeros((128, 128), F32)
            for s in range(NSEG - 1):
                vv = _cat([vT_s[4 * s + c, g * 128:(g + 1) * 128, :] for c in range(4)], 1)
                pp = _cat([pkT_s[4 * s + c, g * 128:(g + 1) * 128, :] for c in range(4)], 1)
                mt = mt + _nt(vv, pp)
                z = jnp.broadcast_to(mt[127:128, :], (16, 128))
                maug_s[(s + 1) * NG + g, 0:128, :] = jnp.where(same, mt, 0.0).astype(BF)
                maug_s[(s + 1) * NG + g, 128:144, :] = jnp.where(zsel, z, 0.0).astype(BF)

    def qm_tile(t0q, hd, qb):
        rows8 = lax.broadcasted_iota(jnp.int32, (8, 128), 0)
        lo, hi = hd.r0 // 2, (hd.r0 + DH) // 2
        t0, t1 = lo // 8, (hi - 1) // 8
        qu = _u32(qT_s[t0q + qb, hd.b + 16 * t0:hd.b + 16 * (t1 + 1), :])
        parts = []
        for t in range(8):
            if t < t0 or t > t1:
                parts.append(jnp.zeros((8, 128), U32))
            else:
                p = qu[(t - t0) * 8:(t - t0 + 1) * 8]
                msk = (rows8 + 8 * t >= lo) & (rows8 + 8 * t < hi)
                parts.append(jnp.where(msk, p, jnp.uint32(0)))
        return _bf(jnp.concatenate(parts, axis=0))

    def vaug(t0q, hd, kb):
        rows8 = lax.broadcasted_iota(jnp.int32, (8, 128), 0)
        vu = _u32(vT_s[t0q + kb, hd.b + hd.a:hd.b + hd.a + 32, :])
        u = hd.r1 // 2
        parts = []
        for t in range(2):
            p = vu[t * 8:(t + 1) * 8]
            if u // 8 == t:
                p = jnp.where(rows8 == (u % 8), jnp.uint32(ONES2), p)
            parts.append(p)
        return _bf(jnp.concatenate(parts, axis=0))

    def stage_a(t0q, hd, kb, slot, qms, mx):
        tri = (lax.broadcasted_iota(jnp.int32, (128, 128), 0)
               <= lax.broadcasted_iota(jnp.int32, (128, 128), 1))
        kt = k_s[hd.g, pl.ds(pl.multiple_of((t0q + kb) * 128, 128), 128), :]
        st = _nn(kt, _cat(qms[kb:], 1))
        for qb in range(kb, 4):
            t = st[:, (qb - kb) * 128:(qb - kb + 1) * 128]
            if qb == kb:
                t = jnp.where(tri, t, NEG)
            s_scr[slot, TILE[(kb, qb)]] = t
            pm = jnp.max(t.reshape(16, 8, 128), axis=0)
            mx[qb] = pm if mx[qb] is None else jnp.maximum(mx[qb], pm)

    def stage_e(qb, slot, mx):
        m = jnp.max(mx[qb], axis=0, keepdims=True)
        for kb in range(qb + 1):
            p_scr[slot, TILE[(kb, qb)]] = jnp.exp2(s_scr[slot, TILE[(kb, qb)]] - m).astype(BF)

    def stage_c(s, t0q, hd, qb, slot):
        p = _cat([p_scr[slot, TILE[(kb, qb)]] for kb in range(qb + 1)], 0)
        acc = _nn(_cat([vaug(t0q, hd, kb) for kb in range(qb + 1)], 1), p)
        rows32 = lax.broadcasted_iota(jnp.int32, (32, 128), 0)
        hrow = (rows32 >= hd.o) & (rows32 < hd.o + DH)
        gt = gate_m[hd.b + hd.r0:hd.b + hd.r0 + 1, :]
        val = acc * ((1.0 - gt) / acc[hd.r1:hd.r1 + 1, :])
        if s > 0:
            nm = nm_s[hd.a:hd.a + 32, qb * 128:(qb + 1) * 128]
            val = val + nm * nm_s[128 + hd.j:129 + hd.j, qb * 128:(qb + 1) * 128]
        pltpu.store(oT_s.at[t0q + qb, hd.b + hd.a:hd.b + hd.a + 32, :], val, mask=hrow)

    def retrieve(s, t0q, g):
        pq = _cat([pqT_s[t0q + qb, g * 128:(g + 1) * 128, :] for qb in range(4)], 1)
        nm = _nn(maug_s[s * NG + g], pq)
        nm_s[0:128, :] = nm[0:128]
        grow = _cat([gate_m[g * 128 + DH * j:g * 128 + DH * j + 1, :] if g * HPG + j < H
                     else jnp.zeros((1, 128), F32) for j in range(8)], 0)
        nm_s[128:136, :] = _cat([grow] * 4, 1) / (nm[128:136] + 1e-6)

    with jax.named_scope("attn"):
        NH = NSEG * H
        mxs = {}
        for t in range(NH + 2):
            na, ne, nc = t, t - 1, t - 2
            if na < NH:
                ha = _Head(na % H)
                qms = [qm_tile(4 * (na // H), ha, qb) for qb in range(4)]
                mxs[na] = [None] * 4
            for i in range(4):
                if na < NH:
                    stage_a(4 * (na // H), ha, i, na % 2, qms, mxs[na])
                if 0 <= ne < NH:
                    stage_e(i, ne % 2, mxs[ne])
                if 0 <= nc < NH:
                    hc = _Head(nc % H)
                    sc = nc // H
                    if i == 0 and hc.j == 0 and sc > 0:
                        retrieve(sc, 4 * sc, hc.g)
                    stage_c(sc, 4 * sc, hc, i, nc % 2)
            mxs.pop(ne, None)

    def out_ln(s, c):
        col = pl.multiple_of((4 * s + c) * 128, 128)
        cs = pl.ds(col, 128)
        hf = h_s[s % 2, c].astype(F32)
        hn = _layernorm_cols(hf).astype(BF)
        hnf = hn.astype(F32)
        r_v[:, cs] = jnp.sum(hnf * wr_m[0:D, :], axis=0, keepdims=True)
        hnT_v[:, cs] = hn
        outT_v[:, cs] = (hf + hnf).astype(BF)

    def out_mm(s, fillers):
        ob = _cat([oT_s[4 * s + c].astype(BF) for c in range(4)], 1)
        for i, (r0, r1) in enumerate(((0, 128), (128, 256), (256, 384), (384, 512), (512, D))):
            a = _nn(woT[r0:r1, :], ob)
            hb = (xT_v[r0:r1, pl.ds(pl.multiple_of(s * L, L), L)].astype(F32) + a).astype(BF)
            for c in range(4):
                h_s[s % 2, c, r0:r1, :] = hb[:, c * 128:(c + 1) * 128]
            if i < len(fillers):
                fillers[i]()

    with jax.named_scope("out"):
        out_mm(0, [])

        def out_body(s, carry):
            out_mm(s + 1, [lambda c=c: out_ln(s, c) for c in range(4)])
            col = pl.multiple_of(s * L, L)
            pltpu.make_async_copy(outT_v.at[:, pl.ds(col, L)], outT_hbm.at[:, pl.ds(col, L)], sem_out.at[s]).start()
            return carry
        lax.fori_loop(0, NSEG - 1, out_body, 0)
        for c in range(4):
            out_ln(NSEG - 1, c)
        cp_out(NSEG - 1).start()

    with jax.named_scope("moe"):
        r = r_v[...]
        rmax_v = jnp.max(r, axis=1, keepdims=True)
        lidx = lax.broadcasted_iota(jnp.int32, (1, S), 1)
        idx = jnp.min(jnp.where(r == rmax_v, lidx, S - 1))
        cb = pl.multiple_of((idx // 128) * 128, 128)
        lane = idx - cb
        rb = pl.multiple_of((lane // 16) * 16, 16)
        hn_blk = hnT_v[:, pl.ds(cb, 128)]
        hn_blk = jnp.concatenate([hn_blk, jnp.zeros((DP - D, 128), BF)], axis=0)
        for kb in range(DP // 128):
            tr_s[:, kb * 128:(kb + 1) * 128] = hn_blk[kb * 128:(kb + 1) * 128, :].T
        xs = tr_s[pl.ds(rb, 16), 0:D]
        cp_wg.wait()
        gt = _nn(xs, wg_v[...])
        cp_wu.wait()
        ut = _nn(xs, wu_v[...])
        mid = (gt * jax.nn.sigmoid(gt) * ut).astype(BF)
        cp_wd.wait()
        y = _nt(mid, wdT_v[...])
        sel = lax.broadcasted_iota(jnp.int32, (16, D), 0) == (lane - rb)
        y = jnp.sum(jnp.where(sel, y, 0.0), axis=0, keepdims=True) * jax.nn.sigmoid(rmax_v)
        y = jnp.concatenate([y, jnp.zeros((1, DP - D), F32)], axis=1)
        yT = jnp.concatenate(
            [jnp.broadcast_to(y[:, kb * 128:(kb + 1) * 128], (128, 128)).T for kb in range(DP // 128)], axis=0)
        for s in range(NSEG):
            cp_out(s).wait()
        old = outT_v[:, pl.ds(cb, 128)].astype(F32)
        lsel = lax.broadcasted_iota(jnp.int32, (D, 128), 1) == lane
        outT_v[:, pl.ds(cb, 128)] = (old + jnp.where(lsel, yT[0:D], 0.0)).astype(BF)
        cp = pltpu.make_async_copy(outT_v.at[:, pl.ds(cb, 128)], outT_hbm.at[:, pl.ds(cb, 128)], sem_out.at[0])
        cp.start()
        cp.wait()


@jax.jit
def pallas_sequential_preLN__memory_aug_infini_attn__moe_arch_mod__prompt_kernel(
        A_x, A_wq, A_wk, A_wv, A_wo, A_beta, B_x, B_w_r, B_w_gate, B_w_up, B_w_down):
    del B_x
    xT = A_x.reshape(S, D).T
    hbm = pl.BlockSpec(memory_space=pltpu.HBM)
    vmem = pltpu.VMEM
    outT = pl.pallas_call(
        _kernel,
        out_shape=jax.ShapeDtypeStruct((D, S), BF),
        in_specs=[pl.BlockSpec(memory_space=pltpu.VMEM), pl.BlockSpec(memory_space=pltpu.VMEM)] + [hbm] * 8,
        out_specs=hbm,
        scratch_shapes=[
            vmem((D, S), BF), vmem((D, D), BF), vmem((D, D), BF), vmem((D, D), BF), vmem((D, D), BF),
            vmem((D, F), BF), vmem((D, F), BF), vmem((D, F), BF),
            vmem((3 * DP, DP), BF), vmem((DP, DP), BF), vmem((DP, 128), F32), vmem((DP, 128), F32),
            vmem((2, DP, L), BF), vmem((NG, S, 128), BF),
            vmem((NQB, DP, 128), BF), vmem((NQB, DP, 128), BF), vmem((NQB, DP, 128), BF), vmem((NQB, DP, 128), BF),
            vmem((NQB, DP, 128), F32),
            vmem((136, L), F32), vmem((NSEG * NG, 144, 128), BF),
            vmem((2, 10, 128, 128), F32), vmem((2, 10, 128, 128), BF),
            vmem((D, S), BF), vmem((D, S), BF), vmem((1, S), F32), vmem((128, DP), BF), vmem((2, 4, D, 128), BF),
            pltpu.SemaphoreType.DMA((11,)), pltpu.SemaphoreType.DMA((NSEG,)),
        ],
        compiler_params=pltpu.CompilerParams(vmem_limit_bytes=100 * 1024 * 1024),
        name="infini_moe",
    )(A_beta.reshape(1, H), B_w_r.reshape(1, D), xT, A_wq, A_wk, A_wv, A_wo, B_w_gate, B_w_up, B_w_down.T)
    return outT.T.reshape(1, S, D)
```

```python
import jax
import jax.numpy as jnp
from jax import lax
import jax.experimental.pallas as pl
import jax.experimental.pallas.tpu as pltpu

S = 2048
D = 576
H = 32
DH = 18
NSEG = 4
L = S // NSEG
F = 4608
HPG = 7
NG = 5
DP = 640
GW = HPG * DH
NQB = S // 128
LOG2E = 1.4426950408889634
BF = jnp.bfloat16
F32 = jnp.float32
U32 = jnp.uint32
NEG = -1e30
ONES2 = 0x3F803F80

TILE = {}
for _kb in range(4):
    for _qb in range(_kb, 4):
        TILE[(_kb, _qb)] = len(TILE)


def _nt(a, b):
    return lax.dot_general(a, b, (((1,), (1,)), ((), ())), preferred_element_type=F32)


def _nn(a, b):
    return jnp.dot(a, b, preferred_element_type=F32)


def _bf(x):
    return pltpu.bitcast(x, BF)


def _u32(x):
    return pltpu.bitcast(x, U32)


def _cat(xs, axis):
    return jnp.concatenate(xs, axis=axis) if len(xs) > 1 else xs[0]


def _phi(t):
    return jnp.where(t > 0, t + 1.0, jnp.exp(jnp.minimum(t, 0.0)))


def _layernorm_cols(x):
    m = jnp.mean(x, axis=0, keepdims=True)
    d = x - m
    v = jnp.mean(d * d, axis=0, keepdims=True)
    return d * lax.rsqrt(v + 1e-5)


class _Head:
    def __init__(self, h):
        self.h = h
        self.g = h // HPG
        self.j = h % HPG
        self.b = self.g * 128
        self.r0 = DH * self.j
        self.a = (self.r0 // 16) * 16
        self.o = self.r0 - self.a
        self.r1 = self.o + DH


def _kernel(beta_ref, wr_ref,
            xT_hbm, wq_hbm, wk_hbm, wv_hbm, wo_hbm, wg_hbm, wu_hbm, wdT_hbm,
            outT_hbm,
            xT_v, wq_v, wk_v, wv_v, wo_v, wg_v, wu_v, wdT_v,
            wT, woT, gate_m, wr_m,
            xnT_s, k_s, qT_s, pqT_s, pkT_s, vT_s, oT_s,
            nm_s, maug_s, s_scr, p_scr,
            hnT_v, outT_v, r_v, tr_s, h_s, h2_s, hsum_s,
            sem_in, sem_out):

    def cp_x(s):
        return pltpu.make_async_copy(xT_hbm.at[:, pl.ds(s * L, L)], xT_v.at[:, pl.ds(s * L, L)], sem_in.at[s])
    cp_wq = pltpu.make_async_copy(wq_hbm, wq_v, sem_in.at[4])
    cp_wk = pltpu.make_async_copy(wk_hbm, wk_v, sem_in.at[5])
    cp_wv = pltpu.make_async_copy(wv_hbm, wv_v, sem_in.at[6])
    cp_wo = pltpu.make_async_copy(wo_hbm, wo_v, sem_in.at[7])
    cp_wg = pltpu.make_async_copy(wg_hbm, wg_v, sem_in.at[8])
    cp_wu = pltpu.make_async_copy(wu_hbm, wu_v, sem_in.at[9])
    cp_wd = pltpu.make_async_copy(wdT_hbm, wdT_v, sem_in.at[10])
    cp_x(0).start()
    cp_wq.start()
    cp_wk.start()
    cp_wv.start()
    for s in range(1, NSEG):
        cp_x(s).start()
    cp_wo.start()

    def cp_out(s):
        return pltpu.make_async_copy(outT_v.at[:, pl.ds(s * L, L)], outT_hbm.at[:, pl.ds(s * L, L)], sem_out.at[s])

    xnT_s[:, D:DP, :] = jnp.zeros((2, DP - D, L), BF)
    zpad = jnp.zeros((NQB, 48, 128), BF)
    qT_s[:, 4 * 128 + 80:5 * 128, :] = zpad
    pqT_s[:, 4 * 128 + 80:5 * 128, :] = zpad
    pkT_s[:, 4 * 128 + 80:5 * 128, :] = zpad
    vT_s[:, 4 * 128 + 80:5 * 128, :] = jnp.ones((NQB, 48, 128), BF)
    for g in range(NG - 1):
        oT_s[:, g * 128 + 120:(g + 1) * 128, :] = jnp.zeros((NQB, 8, 128), F32)
    oT_s[:, 4 * 128 + 64:5 * 128, :] = jnp.zeros((NQB, 64, 128), F32)
    maug_s[0:NG] = jnp.zeros((NG, 144, 128), BF)

    gate = jax.nn.sigmoid(beta_ref[...].astype(F32))
    rows = lax.broadcasted_iota(jnp.int32, (128, 128), 0)
    for g in range(NG):
        gm = jnp.zeros((128, 128), F32)
        for j in range(HPG):
            h = g * HPG + j
            if h < H:
                sel = (rows >= DH * j) & (rows < DH * (j + 1))
                gm = jnp.where(sel, jnp.broadcast_to(gate[:, h:h + 1], (128, 128)), gm)
        gate_m[g * 128:(g + 1) * 128, :] = gm

    wr_row = wr_ref[...].astype(F32)
    wr_row = jnp.concatenate([wr_row, jnp.zeros((1, DP - D), F32)], axis=1)
    for kb in range(DP // 128):
        wr_m[kb * 128:(kb + 1) * 128, :] = jnp.broadcast_to(wr_row[:, kb * 128:(kb + 1) * 128], (128, 128)).T

    def gap_block(w, g):
        c0 = (GW * g // 128) * 128
        c1 = min(c0 + 256, D)
        w = w[:, c0:c1]
        if g < NG - 1:
            return w[:, GW * g - c0:GW * g - c0 + 128]
        rem = D - GW * g
        return jnp.concatenate([w[:, GW * g - c0:], jnp.zeros((D, 128 - rem), BF)], axis=1)

    def transpose_store(w_ref, base, g):
        blk = gap_block(w_ref, g)
        blk = jnp.concatenate([blk, jnp.zeros((DP - D, 128), BF)], axis=0)
        for kb in range(DP // 128):
            wT[base + g * 128:base + (g + 1) * 128, kb * 128:(kb + 1) * 128] = (
                blk[kb * 128:(kb + 1) * 128, :].T)

    def relayout_wo(g):
        n = GW if g < NG - 1 else D - GW * g
        a0 = (GW * g // 16) * 16
        a1 = min(a0 + 144, D)
        wo = wo_v[a0:a1, :].astype(F32)
        blk = wo[GW * g - a0:GW * g - a0 + n, :]
        blk = jnp.concatenate([blk, jnp.zeros((128 - n, D), F32)], axis=0)
        blk = jnp.concatenate([blk, jnp.zeros((128, DP - D), F32)], axis=1).astype(BF)
        for kb in range(DP // 128):
            woT[kb * 128:(kb + 1) * 128, g * 128:(g + 1) * 128] = blk[:, kb * 128:(kb + 1) * 128].T

    def ln1(s, slot, c):
        xr = xT_v[:, pl.ds(pl.multiple_of(s * L + c * 128, 128), 128)].astype(F32)
        xnT_s[slot, 0:D, c * 128:(c + 1) * 128] = _layernorm_cols(xr).astype(BF)

    def proj(s, slot, first, fillers):
        xn = xnT_s[slot]
        rows128 = lax.broadcasted_iota(jnp.int32, (128, L), 0)

        def tiles(g):
            nr = 128 if g < NG - 1 else 80
            return nr, slice(g * 128, g * 128 + nr)

        def do_q(g):
            nr, r = tiles(g)
            q = _nn(wT[g * 128:g * 128 + nr, :], xn)
            qs = (q * (LOG2E * DH ** -0.5)).astype(BF)
            pq = _phi(q).astype(BF)
            for c in range(L // 128):
                cs = slice(c * 128, (c + 1) * 128)
                qT_s[s * 4 + c, r, :] = qs[:, cs]
                pqT_s[s * 4 + c, r, :] = pq[:, cs]

        def do_k(g):
            nr, r = tiles(g)
            k = _nn(wT[DP + g * 128:DP + g * 128 + nr, :], xn)
            pk = _phi(k).astype(BF)
            kb16 = k.astype(BF)
            if nr < 128:
                kb16 = jnp.concatenate([kb16, jnp.zeros((128 - nr, L), BF)], axis=0)
            for c in range(L // 128):
                cs = slice(c * 128, (c + 1) * 128)
                pkT_s[s * 4 + c, r, :] = pk[:, cs]
                k_s[g, pl.ds(pl.multiple_of((s * 4 + c) * 128, 128), 128), :] = kb16[:, cs].T

        def do_v(g):
            nr, r = tiles(g)
            v = _nn(wT[2 * DP + g * 128:2 * DP + g * 128 + nr, :], xn)
            if nr == 128:
                v = jnp.where(rows128 >= GW, 1.0, v)
            v = v.astype(BF)
            for c in range(L // 128):
                vT_s[s * 4 + c, r, :] = v[:, c * 128:(c + 1) * 128]

        for fn, cp, w_ref, base in ((do_q, cp_wq, wq_v, 0), (do_k, cp_wk, wk_v, DP), (do_v, cp_wv, wv_v, 2 * DP)):
            if first:
                cp.wait()
            for g in range(NG):
                if first:
                    transpose_store(w_ref, base, g)
                fn(g)
                f = fillers.get((base // DP) * NG + g)
                if f is not None:
                    f()

    cp_x(0).wait()
    for c in range(4):
        ln1(0, 0, c)
    with jax.named_scope("proj"):
        fillers = {9: lambda: [cp_x(i).wait() for i in range(1, NSEG)]}
        for c in range(4):
            fillers[10 + c] = lambda c=c: ln1(1, 1, c)
        fillers[14] = lambda: (cp_wg.start(), cp_wu.start(), cp_wd.start())
        proj(0, 0, True, fillers)
        cp_wo.wait()

        def proj_body(s, carry):
            nxt = jnp.minimum(s + 1, NSEG - 1)
            fl = {}
            for c in range(4):
                fl[8 + c] = lambda c=c: ln1(nxt, 1 - s % 2, c)
            proj(s, s % 2, False, fl)
            return carry
        lax.fori_loop(1, NSEG, proj_body, 0)
        for g in range(NG):
            relayout_wo(g)

    with jax.named_scope("mem"):
        rr = lax.broadcasted_iota(jnp.int32, (128, 128), 0)
        ll = lax.broadcasted_iota(jnp.int32, (128, 128), 1)
        same = jnp.zeros((128, 128), jnp.bool_)
        zsel = jnp.zeros((16, 128), jnp.bool_)
        r16 = lax.broadcasted_iota(jnp.int32, (16, 128), 0)
        l16 = lax.broadcasted_iota(jnp.int32, (16, 128), 1)
        for j in range(HPG):
            lo, hi = DH * j, DH * (j + 1)
            same = same | ((rr >= lo) & (rr < hi) & (ll >= lo) & (ll < hi))
            zsel = zsel | ((r16 == j) & (l16 >= lo) & (l16 < hi))
        for g in range(NG):
            mt = jnp.zeros((128, 128), F32)
            for s in range(NSEG - 1):
                vv = _cat([vT_s[4 * s + c, g * 128:(g + 1) * 128, :] for c in range(4)], 1)
                pp = _cat([pkT_s[4 * s + c, g * 128:(g + 1) * 128, :] for c in range(4)], 1)
                mt = mt + _nt(vv, pp)
                z = jnp.broadcast_to(mt[127:128, :], (16, 128))
                maug_s[(s + 1) * NG + g, 0:128, :] = jnp.where(same, mt, 0.0).astype(BF)
                maug_s[(s + 1) * NG + g, 128:144, :] = jnp.where(zsel, z, 0.0).astype(BF)

    def qm_tile(t0q, hd, qb):
        rows8 = lax.broadcasted_iota(jnp.int32, (8, 128), 0)
        lo, hi = hd.r0 // 2, (hd.r0 + DH) // 2
        t0, t1 = lo // 8, (hi - 1) // 8
        qu = _u32(qT_s[t0q + qb, hd.b + 16 * t0:hd.b + 16 * (t1 + 1), :])
        parts = []
        for t in range(8):
            if t < t0 or t > t1:
                parts.append(jnp.zeros((8, 128), U32))
            else:
                p = qu[(t - t0) * 8:(t - t0 + 1) * 8]
                msk = (rows8 + 8 * t >= lo) & (rows8 + 8 * t < hi)
                parts.append(jnp.where(msk, p, jnp.uint32(0)))
        return _bf(jnp.concatenate(parts, axis=0))

    def vaug(t0q, hd, kb):
        rows8 = lax.broadcasted_iota(jnp.int32, (8, 128), 0)
        vu = _u32(vT_s[t0q + kb, hd.b + hd.a:hd.b + hd.a + 32, :])
        u = hd.r1 // 2
        parts = []
        for t in range(2):
            p = vu[t * 8:(t + 1) * 8]
            if u // 8 == t:
                p = jnp.where(rows8 == (u % 8), jnp.uint32(ONES2), p)
            parts.append(p)
        return _bf(jnp.concatenate(parts, axis=0))

    def stage_a(t0q, hd, kb, slot, qms, mx):
        tri = (lax.broadcasted_iota(jnp.int32, (128, 128), 0)
               <= lax.broadcasted_iota(jnp.int32, (128, 128), 1))
        kt = k_s[hd.g, pl.ds(pl.multiple_of((t0q + kb) * 128, 128), 128), :]
        st = _nn(kt, _cat(qms[kb:], 1))
        for qb in range(kb, 4):
            t = st[:, (qb - kb) * 128:(qb - kb + 1) * 128]
            if qb == kb:
                t = jnp.where(tri, t, NEG)
            s_scr[slot, TILE[(kb, qb)]] = t
            pm = jnp.max(t.reshape(16, 8, 128), axis=0)
            mx[qb] = pm if mx[qb] is None else jnp.maximum(mx[qb], pm)

    def stage_e(qb, slot, mx):
        m = jnp.max(mx[qb], axis=0, keepdims=True)
        for kb in range(qb + 1):
            p_scr[slot, TILE[(kb, qb)]] = jnp.exp2(s_scr[slot, TILE[(kb, qb)]] - m).astype(BF)

    def stage_c(s, t0q, hd, qb, slot):
        p = _cat([p_scr[slot, TILE[(kb, qb)]] for kb in range(qb + 1)], 0)
        acc = _nn(_cat([vaug(t0q, hd, kb) for kb in range(qb + 1)], 1), p)
        rows32 = lax.broadcasted_iota(jnp.int32, (32, 128), 0)
        hrow = (rows32 >= hd.o) & (rows32 < hd.o + DH)
        gt = gate_m[hd.b + hd.r0:hd.b + hd.r0 + 1, :]
        val = acc * ((1.0 - gt) / acc[hd.r1:hd.r1 + 1, :])
        if s > 0:
            nm = nm_s[hd.a:hd.a + 32, qb * 128:(qb + 1) * 128]
            val = val + nm * nm_s[128 + hd.j:129 + hd.j, qb * 128:(qb + 1) * 128]
        pltpu.store(oT_s.at[t0q + qb, hd.b + hd.a:hd.b + hd.a + 32, :], val, mask=hrow)

    def retrieve(s, t0q, g):
        pq = _cat([pqT_s[t0q + qb, g * 128:(g + 1) * 128, :] for qb in range(4)], 1)
        nm = _nn(maug_s[s * NG + g], pq)
        nm_s[0:128, :] = nm[0:128]
        grow = _cat([gate_m[g * 128 + DH * j:g * 128 + DH * j + 1, :] if g * HPG + j < H
                     else jnp.zeros((1, 128), F32) for j in range(8)], 0)
        nm_s[128:136, :] = _cat([grow] * 4, 1) / (nm[128:136] + 1e-6)

    with jax.named_scope("attn"):
        NH = NSEG * H
        mxs = {}
        for t in range(NH + 2):
            na, ne, nc = t, t - 1, t - 2
            if na < NH:
                ha = _Head(na % H)
                qms = [qm_tile(4 * (na // H), ha, qb) for qb in range(4)]
                mxs[na] = [None] * 4
            for i in range(4):
                if na < NH:
                    stage_a(4 * (na // H), ha, i, na % 2, qms, mxs[na])
                if 0 <= ne < NH:
                    stage_e(i, ne % 2, mxs[ne])
                if 0 <= nc < NH:
                    hc = _Head(nc % H)
                    sc = nc // H
                    if i == 0 and hc.j == 0 and sc > 0:
                        retrieve(sc, 4 * sc, hc.g)
                    stage_c(sc, 4 * sc, hc, i, nc % 2)
            mxs.pop(ne, None)

    def out_ln(s, c):
        cs = pl.ds(pl.multiple_of((4 * s + c) * 128, 128), 128)
        RB = 64
        m = jnp.sum(hsum_s[s % 2, :, c * 128:(c + 1) * 128], axis=0, keepdims=True) * (1.0 / D)
        acc = None
        for i in range(D // RB):
            d = h_s[s % 2, c, i * RB:(i + 1) * RB, :].astype(F32) - m
            t = (d * d).reshape(RB // 8, 8, 128).sum(axis=0)
            acc = t if acc is None else acc + t
        rs = lax.rsqrt(jnp.sum(acc, axis=0, keepdims=True) * (1.0 / D) + 1e-5)
        acc = None
        for i in range(D // RB):
            rr = slice(i * RB, (i + 1) * RB)
            hf = h2_s[s % 2, c, rr, :].astype(F32)
            hn = ((hf - m) * rs).astype(BF)
            hnf = hn.astype(F32)
            t = (hnf * wr_m[rr, :]).reshape(RB // 8, 8, 128).sum(axis=0)
            acc = t if acc is None else acc + t
            hnT_v[rr, cs] = hn
            outT_v[rr, cs] = (hf + hnf).astype(BF)
        r_v[:, cs] = jnp.sum(acc, axis=0, keepdims=True)

    def out_mm(s, fillers):
        ob = _cat([oT_s[4 * s + c].astype(BF) for c in range(4)], 1)
        for i, (r0, r1) in enumerate(((0, 128), (128, 256), (256, 384), (384, 512), (512, D))):
            a = _nn(woT[r0:r1, :], ob)
            hb = (xT_v[r0:r1, pl.ds(pl.multiple_of(s * L, L), L)].astype(F32) + a).astype(BF)
            for c in range(4):
                h_s[s % 2, c, r0:r1, :] = hb[:, c * 128:(c + 1) * 128]
                h2_s[s % 2, c, r0:r1, :] = hb[:, c * 128:(c + 1) * 128]
            t = hb.astype(F32).reshape((r1 - r0) // 8, 8, L).sum(axis=0)
            hsum = t if i == 0 else hsum + t
            if i < len(fillers):
                fillers[i]()
        hsum_s[s % 2] = hsum

    with jax.named_scope("out"):
        out_mm(0, [])

        def out_body(s, carry):
            out_mm(s + 1, [lambda c=c: out_ln(s, c) for c in range(4)])
            col = pl.multiple_of(s * L, L)
            pltpu.make_async_copy(outT_v.at[:, pl.ds(col, L)], outT_hbm.at[:, pl.ds(col, L)], sem_out.at[s]).start()
            return carry
        lax.fori_loop(0, NSEG - 1, out_body, 0)
        for c in range(4):
            out_ln(NSEG - 1, c)
        cp_out(NSEG - 1).start()

    with jax.named_scope("moe"):
        r = r_v[...]
        rmax_v = jnp.max(r, axis=1, keepdims=True)
        lidx = lax.broadcasted_iota(jnp.int32, (1, S), 1)
        idx = jnp.min(jnp.where(r == rmax_v, lidx, S - 1))
        cb = pl.multiple_of((idx // 128) * 128, 128)
        lane = idx - cb
        rb = pl.multiple_of((lane // 16) * 16, 16)
        hn_blk = hnT_v[:, pl.ds(cb, 128)]
        hn_blk = jnp.concatenate([hn_blk, jnp.zeros((DP - D, 128), BF)], axis=0)
        for kb in range(DP // 128):
            tr_s[:, kb * 128:(kb + 1) * 128] = hn_blk[kb * 128:(kb + 1) * 128, :].T
        xs = tr_s[pl.ds(rb, 16), 0:D]
        cp_wg.wait()
        gt = _nn(xs, wg_v[...])
        cp_wu.wait()
        ut = _nn(xs, wu_v[...])
        mid = (gt * jax.nn.sigmoid(gt) * ut).astype(BF)
        cp_wd.wait()
        y = _nt(mid, wdT_v[...])
        sel = lax.broadcasted_iota(jnp.int32, (16, D), 0) == (lane - rb)
        y = jnp.sum(jnp.where(sel, y, 0.0), axis=0, keepdims=True) * jax.nn.sigmoid(rmax_v)
        y = jnp.concatenate([y, jnp.zeros((1, DP - D), F32)], axis=1)
        yT = jnp.concatenate(
            [jnp.broadcast_to(y[:, kb * 128:(kb + 1) * 128], (128, 128)).T for kb in range(DP // 128)], axis=0)
        for s in range(NSEG):
            cp_out(s).wait()
        old = outT_v[:, pl.ds(cb, 128)].astype(F32)
        lsel = lax.broadcasted_iota(jnp.int32, (D, 128), 1) == lane
        outT_v[:, pl.ds(cb, 128)] = (old + jnp.where(lsel, yT[0:D], 0.0)).astype(BF)
        cp = pltpu.make_async_copy(outT_v.at[:, pl.ds(cb, 128)], outT_hbm.at[:, pl.ds(cb, 128)], sem_out.at[0])
        cp.start()
        cp.wait()


@jax.jit
def pallas_sequential_preLN__memory_aug_infini_attn__moe_arch_mod__prompt_kernel(
        A_x, A_wq, A_wk, A_wv, A_wo, A_beta, B_x, B_w_r, B_w_gate, B_w_up, B_w_down):
    del B_x
    xT = A_x.reshape(S, D).T
    hbm = pl.BlockSpec(memory_space=pltpu.HBM)
    vmem = pltpu.VMEM
    outT = pl.pallas_call(
        _kernel,
        out_shape=jax.ShapeDtypeStruct((D, S), BF),
        in_specs=[pl.BlockSpec(memory_space=pltpu.VMEM), pl.BlockSpec(memory_space=pltpu.VMEM)] + [hbm] * 8,
        out_specs=hbm,
        scratch_shapes=[
            vmem((D, S), BF), vmem((D, D), BF), vmem((D, D), BF), vmem((D, D), BF), vmem((D, D), BF),
            vmem((D, F), BF), vmem((D, F), BF), vmem((D, F), BF),
            vmem((3 * DP, DP), BF), vmem((DP, DP), BF), vmem((DP, 128), F32), vmem((DP, 128), F32),
            vmem((2, DP, L), BF), vmem((NG, S, 128), BF),
            vmem((NQB, DP, 128), BF), vmem((NQB, DP, 128), BF), vmem((NQB, DP, 128), BF), vmem((NQB, DP, 128), BF),
            vmem((NQB, DP, 128), F32),
            vmem((136, L), F32), vmem((NSEG * NG, 144, 128), BF),
            vmem((2, 10, 128, 128), F32), vmem((2, 10, 128, 128), BF),
            vmem((D, S), BF), vmem((D, S), BF), vmem((1, S), F32), vmem((128, DP), BF), vmem((2, 4, D, 128), BF), vmem((2, 4, D, 128), BF), vmem((2, 8, L), F32),
            pltpu.SemaphoreType.DMA((11,)), pltpu.SemaphoreType.DMA((NSEG,)),
        ],
        compiler_params=pltpu.CompilerParams(vmem_limit_bytes=100 * 1024 * 1024),
        name="infini_moe",
    )(A_beta.reshape(1, H), B_w_r.reshape(1, D), xT, A_wq, A_wk, A_wv, A_wo, B_w_gate, B_w_up, B_w_down.T)
    return outT.T.reshape(1, S, D)
```
